```python
import os as _os
_os.environ.setdefault('JAX_PLATFORMS', 'cpu')
import jax
import jax.numpy as jnp

def _softmax(x, axis=-1):
    return jax.nn.softmax(x, axis=axis)

def _gelu(x):
    return jax.nn.gelu(x, approximate=True)

def _silu(x):
    return jax.nn.silu(x)

def _sigmoid(x):
    return jax.nn.sigmoid(x)

def _layernorm(x, axis=-1, eps=1e-05):
    m = jnp.mean(x, axis=axis, keepdims=True)
    v = jnp.var(x, axis=axis, keepdims=True)
    return (x - m) / jnp.sqrt(v + eps)

def _scatter_add(tgt, idx, src, axis=0):
    return tgt.at[idx].add(src)

def _segment_sum(src, seg, n):
    return jax.ops.segment_sum(src, seg, n)

class _Rng:

    def __init__(self, key):
        self._k = key

    def _next(self):
        self._k, sub = jax.random.split(self._k)
        return sub

    def normal(self, shape):
        return jax.random.normal(self._next(), shape, dtype=jnp.bfloat16)

    def randint(self, lo, hi, shape):
        return jax.random.randint(self._next(), shape, lo, hi, dtype=jnp.int32)

    def uniform(self, shape, lo=0.0, hi=1.0):
        return jax.random.uniform(self._next(), shape, jnp.bfloat16, lo, hi)

    def permutation(self, n):
        return jax.random.permutation(self._next(), n)
kernel_name = 'sequential_preLN__memory_aug_recurrent_mem_tr__mixer_token_mlp__prompt'

def setup_inputs():
    _rng = _Rng(jax.random.key(int.from_bytes(__import__("os").urandom(4), "little")))
    _w = lambda a: (lambda t: t.astype(jnp.bfloat16) if jnp.issubdtype(t.dtype, jnp.floating) else t)(jnp.asarray(a))

    def _A_setup():
        B, S, Dm = (1, 2048, 448)
        H, Dh = (16, 256)
        M, seg = (8, 32)
        seg = min(seg, S)
        S = S // seg * seg
        return {'x': _w((lambda *s: _rng.normal(s) * 0.05)(B, S, Dm)), 'mem0': _w((lambda *s: _rng.normal(s) * 0.2)(B, M, Dm)), 'Wq': _w((lambda *s: _rng.normal(s) * 1.6)(Dm, H, Dh) * Dm ** (-0.5)), 'Wk': _w((lambda *s: _rng.normal(s) * 1.6)(Dm, H, Dh) * Dm ** (-0.5)), 'Wv': _w((lambda *s: _rng.normal(s) * 0.2)(Dm, H, Dh) * Dm ** (-0.5)), 'Wo': _w((lambda *s: _rng.normal(s) * 0.2)(H, Dh, Dm) * (H * Dh) ** (-0.5)), 'seg_len': seg}
    _A_in = _A_setup()

    def _B_setup():
        B, S, D, F = (1, 2048, 448, 1792)
        return {'x': _w((lambda *s: _rng.normal(s) * 0.05)(B, S, D)), 'w1': _w((lambda *s: _rng.normal(s) * 0.2)(S, F) * S ** (-0.5)), 'b1': _w((lambda *s: _rng.normal(s) * 0.2)(F) * 0.02), 'w2': _w((lambda *s: _rng.normal(s) * 0.2)(F, S) * F ** (-0.5)), 'b2': _w((lambda *s: _rng.normal(s) * 0.05)(S) * 0.02)}
    _B_in = _B_setup()
    return {'A_x': _A_in['x'], 'A_mem0': _A_in['mem0'], 'A_Wq': _A_in['Wq'], 'A_Wk': _A_in['Wk'], 'A_Wv': _A_in['Wv'], 'A_Wo': _A_in['Wo'], 'A_seg_len': _A_in['seg_len'], 'B_x': _B_in['x'], 'B_w1': _B_in['w1'], 'B_b1': _B_in['b1'], 'B_w2': _B_in['w2'], 'B_b2': _B_in['b2']}

def reference(A_x, A_mem0, A_Wq, A_Wk, A_Wv, A_Wo, A_seg_len, B_x, B_w1, B_b1, B_w2, B_b2):

    def _A_ref(x, mem0, Wq, Wk, Wv, Wo, seg_len):
        B, S, Dm = x.shape
        H, Dh = (Wq.shape[1], Wq.shape[2])
        M = mem0.shape[1]
        scale = Dh ** (-0.5)
        n_seg = S // seg_len
        L = M + seg_len
        idx = jnp.arange(L)
        mask = (idx[:, None] < M) | (idx[:, None] >= idx[None, :])
        mem = mem0
        outs = []
        for s in range(n_seg):
            xs = x[:, s * seg_len:(s + 1) * seg_len, :].copy()
            h = jnp.concatenate([mem, xs], axis=1)
            q = jnp.einsum('btd,dhe->bhte', h, Wq)
            k = jnp.einsum('btd,dhe->bhte', h, Wk)
            v = jnp.einsum('btd,dhe->bhte', h, Wv)
            scores = jnp.einsum('bhqe,bhke->bhqk', q, k) * scale
            scores = jnp.where(mask[None, None], scores, -1000000000.0)
            p = _softmax(scores, axis=-1)
            o = jnp.einsum('bhqk,bhke->bhqe', p, v)
            o = jnp.einsum('bhte,hed->btd', o, Wo)
            mem = o[:, :M, :].copy()
            outs.append(o[:, M:, :])
        return jnp.concatenate(outs, axis=1)

    def _B_ref(x, w1, b1, w2, b2):
        B, S, D = x.shape
        h = _layernorm(x, axis=-1)
        u = jnp.einsum('bsd,sf->bdf', h, w1) + b1
        u = _gelu(u)
        y = jnp.einsum('bdf,fs->bds', u, w2) + b2
        return (lambda x, *d: x.transpose(*d))(y, 0, 2, 1)
    x = A_x
    h = x + _A_ref(_layernorm(x, axis=-1), A_mem0, A_Wq, A_Wk, A_Wv, A_Wo, A_seg_len)
    h2 = h + _B_ref(_layernorm(h, axis=-1), B_w1, B_b1, B_w2, B_b2)
    return h2
```

```python
import functools

import jax
import jax.numpy as jnp
from jax import lax
from jax.experimental import pallas as pl
from jax.experimental.pallas import tpu as pltpu

F32 = jnp.float32
BF16 = jnp.bfloat16
U32 = jnp.uint32
LANE = 128
EPS = 1e-5
NEG = -1000000000.0

_NN = (((1,), (0,)), ((), ()))
_NT = (((1,), (1,)), ((), ()))


def _dot(a, b, dims=_NN):
    return lax.dot_general(a, b, dims, preferred_element_type=F32)


def _layernorm_t(v):
    m = jnp.mean(v, axis=0, keepdims=True)
    c = v - m
    var = jnp.mean(c * c, axis=0, keepdims=True)
    return c * lax.rsqrt(var + EPS)


def _gelu(u):
    c = 0.7978845608028654
    return 0.5 * u * (1.0 + jnp.tanh(c * (u + 0.044715 * (u * u * u))))


def _lo_f32(w):
    return pltpu.bitcast(w << 16, F32)


def _hi_f32(w):
    return pltpu.bitcast(w & jnp.uint32(0xFFFF0000), F32)


def _pack(v):
    return pltpu.bitcast(v.astype(BF16), U32)


def _unpack(w):
    return pltpu.bitcast(w, BF16)


def make_kernel(S, D, H, E, M, L, F, cfg):
    DM = (D // LANE) * LANE
    DR = D - DM
    DP = DM + LANE
    NT = DM // LANE
    NP = H // 2
    R = M + L
    JT = R // M
    WC = NT * H * LANE + NP * LANE
    NS = S // L
    assert DR * 2 == LANE and M == 8 and H * M == LANE and E == 2 * LANE
    UNROLL = cfg.get("unroll", 1)
    XR = S // NP
    GC = cfg.get("gchunk", 512)
    scope = jax.named_scope

    def kernel(xt_hbm, mem0_hbm, wq_hbm, wk_hbm, wv_hbm, wo_hbm, w1_hbm, b1_hbm, w2_hbm, b2_hbm,
               out_hbm,
               raw_v, raw_q, raw_k, wo_v, sv, sq, sk, wu, wz, xt_v, xn, o_v, ht_v, kmat, vmat,
               w1_v, w2_v, g_v, hn_v, out_v, mem0_v, b1_v, b2_v, sems, osems):
        cp_v = pltpu.make_async_copy(wv_hbm, raw_v, sems.at[0])
        cp_o = pltpu.make_async_copy(wo_hbm, wo_v, sems.at[1])
        cp_q = pltpu.make_async_copy(wq_hbm, raw_q, sems.at[2])
        cp_k = pltpu.make_async_copy(wk_hbm, raw_k, sems.at[3])
        cp_x = pltpu.make_async_copy(xt_hbm, xt_v, sems.at[4])
        cp_1 = pltpu.make_async_copy(w1_hbm, w1_v, sems.at[5])
        cp_2 = pltpu.make_async_copy(w2_hbm, w2_v, sems.at[6])
        cp_m = pltpu.make_async_copy(mem0_hbm, mem0_v, sems.at[7])
        cp_b1 = pltpu.make_async_copy(b1_hbm, b1_v, sems.at[8])
        cp_b2 = pltpu.make_async_copy(b2_hbm, b2_v, sems.at[9])
        cp_v.start()
        cp_o.start()
        cp_m.start()
        cp_b1.start()
        cp_b2.start()

        lane = lax.broadcasted_iota(jnp.int32, (1, LANE), 1)
        low = lane < DR

        def relayout(raw, dst):
            n = 1024

            def body(c, carry):
                r0 = pl.multiple_of(c * n, n)
                u = pltpu.bitcast(raw[pl.ds(r0, n), :], U32)
                q0 = pl.multiple_of(c * (n // 2), n // 2)
                dst[0, pl.ds(q0, n // 2), :] = u[:, :LANE]
                dst[1, pl.ds(q0, n // 2), :] = u[:, LANE:]
                return carry

            lax.fori_loop(0, D * H // n, body, 0)

        def pair(src, p):
            a = src[0, pl.ds(p, D, stride=NP), :]
            b = src[1, pl.ds(p, D, stride=NP), :]
            return jnp.concatenate([a, b], axis=1)

        def store_folded(dst, p, r0, r1):
            w0, w1 = _pack(r0), _pack(r1)
            for t in range(NT):
                dst[t * NP + p, :, 0:LANE] = w0[:, t * LANE:(t + 1) * LANE]
                dst[t * NP + p, :, LANE:2 * LANE] = w1[:, t * LANE:(t + 1) * LANE]
            rem = jnp.where(low, w0[:, DM:], w1[:, DM:])
            dst[NT * NP + p // 2, :, pl.ds(pl.multiple_of((p % 2) * LANE, LANE), LANE)] = rem

        with scope("wait_v"):
            cp_v.wait()
        cp_q.start()
        with scope("relayout_v"):
            relayout(raw_v, sv)
        with scope("wait_o"):
            cp_o.wait()
        cp_k.start()

        def fold_z(p, carry):
            w = pair(sv, p)
            res = []
            for par, lhs in enumerate((_lo_f32(w), _hi_f32(w))):
                o = wo_v[2 * p + par]
                o = jnp.concatenate([o, o[DM:]], axis=0)
                res.append(_dot(lhs, o, _NT))
            store_folded(wz, p, *res)
            return carry

        with scope("fold_z"):
            lax.fori_loop(0, NP, fold_z, 0)

        with scope("relayout_qk"):
            cp_q.wait()
            cp_x.start()
            relayout(raw_q, sq)
            cp_k.wait()
            cp_1.start()
            relayout(raw_k, sk)
            cp_x.wait()
        cp_2.start()

        scale = float(E) ** -0.5

        def fold_u(p, carry):
            wk = pair(sk, p)
            wq = pair(sq, p)
            res = []
            for lhs, rhs in ((_lo_f32(wk), _lo_f32(wq)), (_hi_f32(wk), _hi_f32(wq))):
                rhs = rhs.astype(BF16)
                rhs = jnp.concatenate([rhs, rhs[DM:]], axis=0)
                res.append(_dot(lhs, rhs, _NT) * scale)
            store_folded(wu, p, *res)
            r0 = pl.multiple_of(p * XR, XR)
            xv = _layernorm_t(xt_v[:, pl.ds(r0, XR)].astype(F32))
            xn[pl.ds(r0, XR), :] = jnp.concatenate([xv, xv[DM:]], axis=0).T
            return carry

        with scope("fold_u"):
            lax.fori_loop(0, NP, fold_u, 0)

        row = lax.broadcasted_iota(jnp.int32, (R, LANE), 0)
        l2 = lax.broadcasted_iota(jnp.int32, (R, LANE), 1)
        jlo = l2 & (M - 1)

        def group_all(v, op):
            k = 1
            while k < M:
                up = pltpu.roll(v, k, 1)
                dn = pltpu.roll(v, LANE - k, 1)
                v = op(v, jnp.where((l2 & k) == 0, dn, up))
                k *= 2
            return v

        def project(hk, w_ref, dst):
            nb = GC // (2 * LANE)
            for t in range(NT):
                for p0 in range(0, NP, nb):
                    w = jnp.concatenate([w_ref[t * NP + p0 + i] for i in range(nb)], axis=1)
                    r = _dot(hk, _unpack(w))
                    for jt in range(JT):
                        rows = r[jt * M:(jt + 1) * M]
                        blk = jnp.concatenate(
                            [rows[:, i * LANE:(i + 1) * LANE] for i in range(2 * nb)], axis=0)
                        dst[pl.ds(jt * (LANE // 2) + p0 * M, nb * M), t * LANE:(t + 1) * LANE] = _pack(blk)
            for q0 in range(0, NP // 2, nb):
                w = jnp.concatenate([w_ref[NT * NP + q0 + i] for i in range(nb)], axis=1)
                r = _dot(hk, _unpack(w))
                for jt in range(JT):
                    rows = r[jt * M:(jt + 1) * M]
                    pieces = []
                    for i in range(2 * nb):
                        tile = rows[:, i * LANE:(i + 1) * LANE]
                        pieces.append(jnp.where(low, tile, 0.0))
                        pieces.append(jnp.where(low, 0.0, tile))
                    blk = jnp.concatenate(pieces, axis=0)
                    dst[pl.ds(jt * (LANE // 2) + 2 * q0 * M, 2 * nb * M), DM:DP] = _pack(blk)

        def step(s, mem):
            r0 = pl.multiple_of(s * L, L)
            hh = jnp.concatenate([mem, xn[pl.ds(r0, L), :]], axis=0)
            hk = hh[:, :D]
            project(hk, wu, kmat)
            sc = _dot(hh, _unpack(kmat[...]), _NT)
            project(hk, wz, vmat)
            tiles = []
            for jt in range(JT):
                ok = (row < M) | (row >= jlo + jt * M)
                tiles.append(jnp.where(ok, sc[:, jt * LANE:(jt + 1) * LANE], NEG))
            mx = functools.reduce(jnp.maximum, tiles)
            mx = group_all(mx, jnp.maximum)
            ex = [jnp.exp(t - mx) for t in tiles]
            den = group_all(functools.reduce(jnp.add, ex), jnp.add)
            inv = 1.0 / den
            pm = jnp.concatenate([e * inv for e in ex], axis=1)
            o = _dot(pm, _unpack(vmat[...]))
            t = o[:, DM:]
            t = t + pltpu.roll(t, DR, 1)
            o = jnp.concatenate([o[:, :DM], t], axis=1)
            o_v[pl.ds(r0, L), :] = o[M:]
            return o[:M]

        def steps(i, mem):
            for j in range(UNROLL):
                mem = step(i * UNROLL + j, mem)
            return mem

        cp_m.wait()
        m0 = mem0_v[...].astype(F32)
        with scope("recurrence"):
            lax.fori_loop(0, NS // UNROLL, steps, jnp.concatenate([m0, m0[:, DM:]], axis=1))

        TB = 256

        def norm_block(i, carry):
            r0 = pl.multiple_of(i * TB, TB)
            ht = xt_v[:, pl.ds(r0, TB)].astype(F32) + o_v[pl.ds(r0, TB), :].T[:D]
            ht_v[:, pl.ds(r0, TB)] = ht
            hn_v[:, pl.ds(r0, TB)] = _layernorm_t(_layernorm_t(ht)).astype(BF16)
            return carry

        with scope("norm"):
            lax.fori_loop(0, S // TB, norm_block, 0)
        cp_1.wait()
        cp_b1.wait()
        cp_b2.wait()

        FC = 256
        b1 = b1_v[...].astype(F32).reshape(1, F)
        b2 = b2_v[...].astype(F32).reshape(1, S)

        with scope("mlp1"):
            for j in range(F // FC):
                c0 = j * FC
                u = _dot(hn_v[...], w1_v[:, pl.ds(c0, FC)]) + b1[:, c0:c0 + FC]
                g_v[:, pl.ds(c0, FC)] = _gelu(u).astype(BF16)
        cp_2.wait()

        SC = 256

        def out_copy(j):
            r0 = j * SC
            return pltpu.make_async_copy(out_v.at[:, pl.ds(r0, SC)], out_hbm.at[:, pl.ds(r0, SC)], osems.at[j])

        with scope("mlp2"):
            for j in range(S // SC):
                c0 = j * SC
                y = _dot(g_v[...], w2_v[:, pl.ds(c0, SC)]) + b2[:, c0:c0 + SC]
                out_v[:, pl.ds(c0, SC)] = (ht_v[:, pl.ds(c0, SC)] + y).astype(BF16)
                out_copy(j).start()
        with scope("tail"):
            for j in range(S // SC):
                out_copy(j).wait()

    scratch = [
        pltpu.VMEM((D * H, E), BF16), pltpu.VMEM((D * H, E), BF16), pltpu.VMEM((D * H, E), BF16),
        pltpu.VMEM((H, D, E), BF16),
        pltpu.VMEM((2, D * NP, LANE), U32), pltpu.VMEM((2, D * NP, LANE), U32),
        pltpu.VMEM((2, D * NP, LANE), U32),
        pltpu.VMEM((WC // (2 * LANE), D // 2, 2 * LANE), U32),
        pltpu.VMEM((WC // (2 * LANE), D // 2, 2 * LANE), U32),
        pltpu.VMEM((D, S), BF16), pltpu.VMEM((S, DP), F32), pltpu.VMEM((S, DP), F32),
        pltpu.VMEM((D, S), F32),
        pltpu.VMEM((JT * LANE // 2, DP), U32), pltpu.VMEM((JT * LANE // 2, DP), U32),
        pltpu.VMEM((S, F), BF16), pltpu.VMEM((F, S), BF16),
        pltpu.VMEM((D, F), BF16), pltpu.VMEM((D, S), BF16), pltpu.VMEM((D, S), BF16),
        pltpu.VMEM((M, D), BF16), pltpu.VMEM((F,), BF16), pltpu.VMEM((S,), BF16),
        pltpu.SemaphoreType.DMA((10,)), pltpu.SemaphoreType.DMA((S // 256,)),
    ]
    return kernel, scratch


def build(cfg):
    @functools.partial(jax.jit, static_argnames=("A_seg_len",))
    def fn(A_x, A_mem0, A_Wq, A_Wk, A_Wv, A_Wo, A_seg_len, B_x, B_w1, B_b1, B_w2, B_b2):
        del B_x
        _, S, D = A_x.shape
        _, H, E = A_Wq.shape
        M = A_mem0.shape[1]
        F = B_w1.shape[1]
        kernel, scratch = make_kernel(S, D, H, E, M, A_seg_len, F, cfg)
        hbm = pl.BlockSpec(memory_space=pltpu.HBM)
        out = pl.pallas_call(
            kernel,
            out_shape=pltpu.HBM((D, S), A_x.dtype),
            in_specs=[hbm] * 10,
            out_specs=hbm,
            scratch_shapes=scratch,
            compiler_params=pltpu.CompilerParams(vmem_limit_bytes=110 * 1024 * 1024),
        )(A_x.reshape(S, D).T, A_mem0.reshape(M, D), A_Wq.reshape(D * H, E), A_Wk.reshape(D * H, E),
          A_Wv.reshape(D * H, E), A_Wo.transpose(0, 2, 1), B_w1, B_b1, B_w2, B_b2)
        return out.T.reshape(A_x.shape)

    return fn


pallas_sequential_preLN__memory_aug_recurrent_mem_tr__mixer_token_mlp__prompt_kernel = build({})
```

```python
import contextlib
import functools

import jax
import jax.numpy as jnp
from jax import lax
from jax.experimental import pallas as pl
from jax.experimental.pallas import tpu as pltpu

F32 = jnp.float32
BF16 = jnp.bfloat16
U32 = jnp.uint32
LANE = 128
EPS = 1e-5
LOG2E = 1.4426950408889634
NEG = -1000000000.0

_dot = functools.partial(lax.dot_general, dimension_numbers=(((1,), (0,)), ((), ())),
                         preferred_element_type=F32)
_dot_nt = functools.partial(lax.dot_general, dimension_numbers=(((1,), (1,)), ((), ())),
                            preferred_element_type=F32)


def _layernorm_t(v, gain=None):
    m = jnp.mean(v, axis=0, keepdims=True)
    c = v - m
    var = jnp.mean(c * c, axis=0, keepdims=True)
    inv = lax.rsqrt(var + EPS)
    return c * (inv if gain is None else inv * gain)


def _gelu_of_half(v):
    c = 0.7978845608028654
    return v + v * jnp.tanh(v * (2.0 * c + (8.0 * 0.044715 * c) * (v * v)))


def _lo_f32(w):
    return pltpu.bitcast(w << 16, F32)


def _hi_f32(w):
    return pltpu.bitcast(w & jnp.uint32(0xFFFF0000), F32)


def _pack(v):
    return pltpu.bitcast(v.astype(BF16), U32)


def _interleave(even, odd):
    return pltpu.bitcast(pltpu.pack_elementwise([even, odd], packed_dtype=BF16), U32)


def _unpack(w):
    return pltpu.bitcast(w, BF16)


def make_kernel(S, D, H, E, M, L, F, cfg):
    DM = (D // LANE) * LANE
    DR = D - DM
    DP = DM + LANE
    NT = DM // LANE
    NP = H // 2
    R = M + L
    KT = H * R // LANE
    WB = NT * NP + NP // 2
    NB = S // LANE
    SB = LANE // L
    HP = LANE // 2
    HG = H // 2
    PG = HG // 2
    assert DR * 2 == LANE and M == 8 and H == 16 and R == 40 and E == 2 * LANE
    scope = jax.named_scope if cfg.get('scopes', 0) else (lambda name: contextlib.nullcontext())
    PRE, POST = ([(w[0], int(w[1])) for w in part.split()] for part in
                 cfg.get("plan", "s0 k0 k3 k1 k2 t0 t1 v3|v0 v1 v2").split("|"))
    KCH = cfg.get("kch", (192, 256))
    REV = cfg.get('rev', 1)
    KOFF = [D - sum(KCH[:i + 1]) if REV else sum(KCH[:i]) for i in range(len(KCH))]
    ZW = cfg.get('zw', ((0,), (1,), (2,), (3,)))
    NI_AT = cfg.get('ni', 1)
    LATE = cfg.get('late', 0)
    GU = cfg.get('gu', 1)
    DEEP1 = cfg.get('d1', (1, 4, 3))
    DEEP2 = cfg.get('d2', (1, 4, 6, 3))
    ORD1 = cfg.get('o1', (2, 5, 4, 1, 3, 0, 6))
    ORD2 = cfg.get('o2', (1, 3, 2, 4, 0, 6, 5))
    XS = cfg.get('xs', 2)
    NPEEL = cfg.get('npeel', 0)
    NB_AT = cfg.get('nb', 2)
    SC = cfg.get('sc', 512)
    EARLY = cfg.get('early', {})
    FCH = cfg.get('fch', ((0, 896),))
    NC = D // DR

    TILE = [(0, 1, 4), (2, 3, 5), (8, 9, 12), (10, 11, 13), (6, 7, 14)]
    LAST = H - 1
    KPAIR = [(2, 0), (3, 1), (5, 4), (7, 6)]
    KPOS = {g * HG + j: (g * PG + i, half)
            for g in range(2) for i, pr in enumerate(KPAIR) for half, j in enumerate(pr)}

    ZWAIT = cfg.get('zwait', {0: (0,), 2: (1,), 4: (2, 3)})
    KW = cfg.get('kw', 3)
    QW = cfg.get('qw', 3)
    DEFER = cfg.get('defer', 0)
    ZN = cfg.get('zn', 0)
    ZPIECES = cfg.get('zp', ((0, 448),))
    XW = cfg.get('xw', 0)

    def kernel(xt_hbm, mem0_hbm, wq_hbm, wk_hbm, wv_hbm, wo_hbm, w1_hbm, b1_hbm, w2_hbm, b2_hbm,
               out_hbm,
               raw, raw_k, wo_v, sw, sk, wu, wz, wt, wb, xt_v, xn, o_v, ht_v,
               w1_v, w2_v, g_v, hn_v, out_v, mem0_v, b1_v, b2_v, b2f_v,
               sems, sem_r, sem_o, sem_k, osems):
        def heads(g):
            return pl.ds(pl.multiple_of(g * HG, HG), HG)

        def cp_v(g):
            return pltpu.make_async_copy(wv_hbm.at[:, heads(g), :], raw.at[g], sem_r.at[g])

        def cp_q(g):
            return pltpu.make_async_copy(wq_hbm.at[:, heads(g), :], raw.at[2 + g], sem_r.at[2 + g])

        def cp_k(g, c):
            rows = pl.ds(c * DR, DR)
            return pltpu.make_async_copy(wk_hbm.at[rows, heads(g), :], raw_k.at[g, rows], sem_k.at[g * NC + c])

        def cp_o(p):
            return pltpu.make_async_copy(wo_hbm.at[pl.ds(2 * p, 2)], wo_v.at[pl.ds(2 * p, 2)], sem_o.at[p])

        def cp_x(b):
            cols = pl.ds(pl.multiple_of(b * LANE, LANE), LANE)
            return pltpu.make_async_copy(xt_hbm.at[:, cols], xt_v.at[:, cols], sems.at[b % 2])

        def cp_1(b):
            rows = pl.ds(pl.multiple_of(b * LANE, LANE), LANE)
            return pltpu.make_async_copy(w1_hbm.at[rows], w1_v.at[rows], sems.at[2])

        def cp_2(b):
            rows = pl.ds(pl.multiple_of(b * (F // NB), F // NB), F // NB)
            return pltpu.make_async_copy(w2_hbm.at[rows], w2_v.at[rows], sems.at[3])

        cp_m = pltpu.make_async_copy(mem0_hbm, mem0_v, sems.at[4])
        cp_b1 = pltpu.make_async_copy(b1_hbm, b1_v, sems.at[5])
        cp_b2 = pltpu.make_async_copy(b2_hbm, b2_v, sems.at[6])

        def start_z(g, carry):
            cp_v(g).start()
            lax.fori_loop(0, PG, lambda pp, c: (cp_o(g * PG + pp).start(), c)[1], 0)
            return carry

        def start_u(g, carry):
            cp_q(g).start()
            lax.fori_loop(0, NC, lambda i, c: (cp_k(g, NC - 1 - i if REV else i).start(), c)[1], 0)
            cp_x(g).start()
            return carry

        lax.fori_loop(0, 2, start_z, 0)
        lax.fori_loop(0, 2, start_u, 0)
        for cp in (cp_m, cp_b1, cp_b2):
            cp.start()

        lane = lax.broadcasted_iota(jnp.int32, (1, LANE), 1)
        low = lane < DR
        o_v[0:LANE, :] = jnp.zeros((LANE, DP), F32)

        def relayout(src, dst, d0, nd):
            n = 64
            for d in range(d0, d0 + nd, n):
                u = pltpu.bitcast(src[d:d + n].reshape(n * HG, E), U32)
                dst[0, d * PG:(d + n) * PG, :] = u[:, :LANE]
                dst[1, d * PG:(d + n) * PG, :] = u[:, LANE:]

        def pair(src, pp, d0, nd, step=1):
            idx = pl.ds(d0 * PG + pp, nd, stride=step * PG)
            return jnp.concatenate([src[0, idx, :], src[1, idx, :]], axis=1)

        def store_main(dst, g, j, d0, w):
            rows = pl.ds(d0 // 2, w.shape[0])
            for t in range(NT):
                dst[t * NP + g * PG + j // 2, rows, (j % 2) * LANE:(j % 2 + 1) * LANE] = w[:, t * LANE:(t + 1) * LANE]

        def store_rem(dst, g, i, d0, tile):
            rows = pl.ds(d0 // 2, tile.shape[0] // 2)
            dst[NT * NP + g * (PG // 2) + i // 2, rows, (i % 2) * LANE:(i % 2 + 1) * LANE] = _pack(tile)

        def fold_z(g, carry):
            rem = {}
            for j in range(HG):
                pp, par = divmod(j, 2)
                p = g * PG + pp
                if j in ZWAIT:
                    if True:
                        for i in ZWAIT[j]:
                            cp_o(g * PG + i).wait()
                if par == 0:
                    w = pair(sw.at[g], pp, 0, D)
                    we, wo = pair(sw.at[g], pp, 0, D // 2, 2), pair(sw.at[g], pp, 1, D // 2, 2)
                if j == HG - 1:
                    if True:
                        pltpu.make_async_copy(raw.at[g + 1], raw.at[g + 1], sem_r.at[g + 1]).wait()
                o = wo_v[2 * p + par]
                v = _hi_f32(w) if par else _lo_f32(w)
                rem[j] = _dot_nt(o[DM:], jnp.concatenate([v, v[DM:]], axis=0).astype(BF16))
                half = _hi_f32 if par else _lo_f32
                r = _interleave(_dot_nt(half(we), o[:DM]), _dot_nt(half(wo), o[:DM]))
                if j == HG - 1:
                    relayout(raw.at[g + 1], sw.at[1 - g], 0, D)
                store_main(wz, g, j, 0, r[:DM // 2])
                wb[p, par * (DR // 2):(par + 1) * (DR // 2), :DM] = r[DM // 2:]
                for i, hs in enumerate(KPAIR):
                    if j == max(hs):
                        tile = jnp.concatenate([rem[h] for h in hs], axis=0).T
                        store_rem(wz, g, i, 0, tile[:DM])
                        t0 = tile[DM:D]
                        t1 = pltpu.roll(t0, DR, 1)
                        for h, dup in zip(hs, (jnp.where(low, t0, t1), jnp.where(low, t1, t0))):
                            wb[g * PG + h // 2, (h % 2) * (DR // 2):(h % 2 + 1) * (DR // 2), DM:] = _pack(dup)
            return carry

        with scope("fold_z"):
            if True:
                cp_v(0).wait()
            relayout(raw.at[0], sw.at[0], 0, D)
            lax.fori_loop(0, 2, fold_z, 0)

        scale = float(E) ** -0.5 * LOG2E

        def norm_input(b):
            r0 = pl.multiple_of(b * LANE, LANE)
            xv = _layernorm_t(xt_v[:, pl.ds(r0, LANE)].astype(F32))
            xn[pl.ds(r0, LANE), :] = jnp.concatenate([xv, xv[DM:]], axis=0).T

        def fold_u(g, carry):
            def fetch(c):
                if True:
                    for i in range(KOFF[c] // DR, (KOFF[c] + KCH[c]) // DR):
                        cp_k(g, i).wait()
                relayout(raw_k.at[g], sk, KOFF[c], KCH[c])

            for c, (d0, nd) in enumerate(zip(KOFF, KCH)):
                nm = min(nd, DM - d0)
                rem = {}
                for pp in range(PG):
                    if c == 0 and pp == 0:
                        fetch(0)
                    if c + 1 < len(KCH) and pp == KW:
                        if c + 2 == len(KCH):
                            cp_x(g).wait()
                        fetch(c + 1)
                    if c + 1 == len(KCH) and pp == XW:
                        norm_input(g)
                    wk = pair(sk, pp, d0, nd)
                    ke, ko = pair(sk, pp, d0, nm // 2, 2), pair(sk, pp, d0 + 1, nm // 2, 2)
                    wq = pair(sw.at[g], pp, 0, D)
                    tail = []
                    for par, (k, q) in enumerate(((_lo_f32(wk), _lo_f32(wq)), (_hi_f32(wk), _hi_f32(wq)))):
                        j = 2 * pp + par
                        rem[j] = _dot_nt(q[DM:], k[:nm].astype(BF16)) * scale
                        half = _hi_f32 if par else _lo_f32
                        qm = q[:DM].astype(BF16)
                        cut = (nm + nd) // 2
                        lhs = [half(ke), half(ko)]
                        if nm < nd:
                            lhs = [jnp.concatenate([lhs[0], k[nm:cut]], axis=0),
                                   jnp.concatenate([lhs[1], k[cut:]], axis=0)]
                            qr = jnp.concatenate([q[DM:], q[DM:]], axis=0).astype(BF16)
                            corner = _dot_nt(k[nm:], qr) * scale
                        re, ro = (_dot_nt(a, qm) * scale for a in lhs)
                        store_main(wu, g, j, d0, _interleave(re[:nm // 2], ro[:nm // 2]))
                        if nm < nd:
                            tail.append(jnp.concatenate(
                                [jnp.concatenate([re[nm // 2:], ro[nm // 2:]], axis=0), corner], axis=1))
                        for i, hs in enumerate(KPAIR):
                            if j == max(hs):
                                store_rem(wu, g, i, d0, jnp.concatenate([rem[h] for h in hs], axis=0).T)
                    if tail:
                        wt[g * (PG // 2) + pp // 2, :, (pp % 2) * LANE:(pp % 2 + 1) * LANE] = _pack(
                            jnp.concatenate(tail, axis=0).T[:D])

            @pl.when(g == 0)
            def _():
                if True:
                    cp_q(1).wait()
                relayout(raw.at[3], sw.at[1], 0, D)

            return carry

        with scope("fold_u"):
            lax.fori_loop(0, 2, fold_u, 0)

        def project_tile(ha, w_ref, t):
            base, n = (t * NP, NP) if t < NT else (NT * NP, NP // 2)
            out = []
            for p0 in range(0, n, 2):
                w = jnp.concatenate([w_ref[base + p0], w_ref[base + p0 + 1]], axis=1)
                r = _dot(ha, _unpack(w))
                out += [r[:, i * LANE:(i + 1) * LANE] for i in range(4)]
            return out

        def main_blocks(ha, w_ref, t):
            hd = project_tile(ha, w_ref, t)
            return [jnp.concatenate([hd[h] for h in TILE[k]] + [hd[LAST][k * M:(k + 1) * M]], axis=0)
                    for k in range(KT)]

        def rem_blocks(ha, w_ref, rr):
            rem = project_tile(ha, w_ref, NT)
            blocks = []
            for k in range(KT):
                own = TILE[k][2] % 2
                mine = low if own == 0 else jnp.logical_not(low)

                def part(h):
                    i, half = KPOS[h]
                    v = rem[i]
                    if h == LAST:
                        v = v[k * M:(k + 1) * M]
                    if half == own:
                        v = pltpu.roll(v, DR, 1)
                    return jnp.where(mine, rr if h == TILE[k][2] else 0.0, v)

                blocks.append(jnp.concatenate([part(h) for h in TILE[k]] + [part(LAST)], axis=0))
            return blocks

        key = lax.broadcasted_iota(jnp.int32, (R, 3 * R), 0)
        col = lax.broadcasted_iota(jnp.int32, (R, 3 * R), 1)
        qry = col - jnp.where(col >= R, R, 0) - jnp.where(col >= 2 * R, R, 0)
        grp = lax.broadcasted_iota(jnp.int32, (M, 3 * R), 1)

        def softmax_keys(v):
            v = jnp.where((qry < M) | (qry >= key), v, NEG * LOG2E)
            e = jnp.exp2(v - jnp.max(v, axis=0, keepdims=True))
            den = jnp.sum(e, axis=0, keepdims=True)
            inv = pl.reciprocal(den, approx=True)
            return e * (inv * (2.0 - den * inv))

        def shift(v, n):
            if n == 0:
                return v
            v = jnp.concatenate([v, jnp.zeros((M, LANE - 3 * R), F32)], axis=1)
            return pltpu.roll(v, n % LANE, 1)[:, :3 * R]

        def step(s, mem, side):
            r0 = pl.multiple_of(s * L, L)
            hh = jnp.concatenate([mem, xn[pl.ds(r0, L), :]], axis=0)
            ha, rr = hh[:, :DM], hh[:, DM:]
            own = jnp.concatenate([jnp.where(low, rr, 0.0), jnp.where(low, 0.0, rr),
                                   jnp.zeros((LANE - 2 * R, LANE), F32)], axis=0)
            own_t = own.T
            kb = [None] * (NT + 1)
            vb = [None] * (NT + 1)
            tq = []

            def run(items):
                for kind, t in items:
                    if kind == "k":
                        kb[t] = [b.T for b in (main_blocks(ha, wu, t) if t < NT else rem_blocks(ha, wu, rr))]
                    elif kind == "v":
                        vb[t] = main_blocks(ha, wz, t) if t < NT else rem_blocks(ha, wz, rr)
                    elif kind == "t":
                        r = _dot(hh[:, :D], _unpack(jnp.concatenate([wt[2 * t], wt[2 * t + 1]], axis=1)))
                        tq.extend(r[:, i * LANE:(i + 1) * LANE] for i in range(4))
                    else:
                        side()

            run(PRE)
            sc = []
            for k in range(KT):
                i, half = divmod(TILE[k][2], 2)
                third = jnp.where(low, tq[i], rr) if half == 0 else jnp.where(low, rr, tq[i])
                rhs = jnp.concatenate([kb[t][k] for t in range(NT + 1)] + [own_t], axis=0)
                sc.append(_dot(jnp.concatenate([ha, third, tq[TILE[k][0] // 2]], axis=1), rhs.astype(BF16)))
            sc.append(_dot(tq[LAST // 2], own_t.astype(BF16)))
            run(POST)

            sa = jnp.concatenate(sc[:3], axis=0).T
            sb = jnp.concatenate(sc[3:], axis=0).T
            g1, g3 = grp < R, grp >= 2 * R
            tail = [(sa if k < 3 else sb)[3 * R:] for k in range(KT)]
            home = sb[R:2 * R] + jnp.concatenate(
                [jnp.where(g3, shift(tail[k], (2 - k % 3) * R), 0.0) for k in range(KT)], axis=0)
            ps = [softmax_keys(v) for v in (sa[0:R], sa[R:2 * R], sa[2 * R:3 * R], sb[0:R], home, sb[2 * R:3 * R])]
            back = [shift(ps[4][k * M:(k + 1) * M], (k % 3 - 2) * R) for k in range(KT)]
            ta = jnp.where(g1, back[0], jnp.where(g3, back[2], back[1]))
            tb = jnp.where(g1, back[3], back[4])
            pa = jnp.concatenate(ps[:3] + [ta], axis=0).T
            pb = jnp.concatenate(ps[3:] + [tb], axis=0).T
            pm = [pa[i * R:(i + 1) * R] for i in range(3)] + [pb[i * R:(i + 1) * R] for i in range(3)]

            if XS >= 3:
                rhs = jnp.concatenate([jnp.concatenate([vb[t][k] for t in range(NT)], axis=1) for k in range(KT)], axis=0)
                oa = _dot(jnp.concatenate(pm[:KT], axis=1), rhs.astype(BF16))
            if XS == 0:
                xs = [_dot(pm[k], jnp.concatenate([own, vb[NT][k]], axis=1).astype(BF16)) for k in range(KT)]
            elif XS == 1:
                xs = [jnp.concatenate([_dot(pm[k], own.astype(BF16)), _dot(pm[k], vb[NT][k].astype(BF16))], axis=1)
                      for k in range(KT)]
            elif XS >= 2:
                xa = [_dot(pm[k], own.astype(BF16)) for k in range(KT)]
                xs = [jnp.concatenate([xa[k], _dot(pm[k], vb[NT][k].astype(BF16))], axis=1) for k in range(KT)]
            xl = _dot(pm[KT], own.astype(BF16))
            if XS < 3:
                rhs = jnp.concatenate([jnp.concatenate([vb[t][k] for t in range(NT)], axis=1) for k in range(KT)], axis=0)
                oa = _dot(jnp.concatenate(pm[:KT], axis=1), rhs.astype(BF16))
            src = {TILE[k][2]: xs[k][:, LANE:] for k in range(KT)}
            src[LAST] = xl
            whole = {TILE[k][0] // 2: xs[k][:, :LANE] for k in range(KT)}
            pr = [whole[p] if p in whole else jnp.where(low, src[2 * p], src[2 * p + 1]) for p in range(NP)]
            ob = _dot(jnp.concatenate(pr, axis=1),
                      _unpack(jnp.concatenate([wb[p] for p in range(NP)], axis=0)))
            hi_sum = functools.reduce(jnp.add, [xs[k][:, LANE:] for k in range(KT) if TILE[k][2] % 2 == 0])
            lo_sum = functools.reduce(jnp.add, [xs[k][:, LANE:] for k in range(KT) if TILE[k][2] % 2 == 1])
            orem = jnp.where(low, lo_sum, hi_sum)
            orem = orem + pltpu.roll(orem, DR, 1)
            o = ob + jnp.concatenate([oa, orem], axis=1)
            o_v[pl.ds(r0, L), :] = o[M:]
            return o[:M]

        def norm_block(b):
            cols = pl.ds(pl.multiple_of(b * LANE, LANE), LANE)
            ht = xt_v[:, cols].astype(F32) + o_v[cols, :].T[:D]
            ht_v[:, cols] = ht
            hn_v[:, cols] = _layernorm_t(_layernorm_t(ht), 0.5)

        def block(b, mem):
            @pl.when(b > 0)
            def _():
                cp_1(b - 1).wait()
                cp_2(b - 1).wait()

            @pl.when((b > 0) & (b + 1 < NB))
            def _():
                cp_x(b + 1).wait()

            cp_1(b).start()
            cp_2(b).start()

            @pl.when(b + 2 < NB)
            def _():
                cp_x(b + 2).start()

            for j in range(SB):
                def side():
                    if j == NB_AT:
                        norm_block(jnp.maximum(b - 1, 0))
                    if j == NI_AT:
                        norm_input(jnp.minimum(b + 1, NB - 1))
                mem = step(b * SB + j, mem, side)
            return mem

        for cp in (cp_m, cp_b1, cp_b2):
            cp.wait()
        with scope("recurrence0"):
            m0 = mem0_v[...].astype(F32)
            mem = jnp.concatenate([m0, m0[:, DM:]], axis=1)
        with scope("recurrence"):
            lax.fori_loop(0, NB, block, mem)

        cp_1(NB - 1).wait()
        cp_2(NB - 1).wait()

        DH, FH, SH = D // 2, F // 2, S // 2

        def widen(a, b, sign):
            a, b = a.astype(F32), b.astype(F32)
            return (a + b if sign > 0 else a - b).astype(BF16)

        def operand(quad, spec):
            qa, sign, qb = spec
            return widen(quad(qa), quad(qb), sign) if sign else quad(qa).astype(BF16)

        LHS = ((0, 1, 3), (2, 1, 3), (0, 0, 0), (3, 0, 0), (0, 1, 1), (2, -1, 0), (1, -1, 3))
        RHS = ((0, 1, 3), (0, 0, 0), (1, -1, 3), (2, -1, 0), (3, 0, 0), (0, 1, 1), (2, 1, 3))

        def product(a, b, depth):
            m, k = a.shape
            n = b.shape[1]
            if not depth:
                return _dot(a.astype(BF16), b.astype(BF16))
            mh, kh, nh = m // 2, k // (2 * LANE) * LANE, n // (2 * LANE) * LANE
            af, bf = a.astype(F32), b.astype(F32)

            def aq(q):
                return af[(q // 2) * mh:(q // 2 + 1) * mh, (q % 2) * kh:(q % 2 + 1) * kh]

            def bq(q):
                return bf[(q // 2) * kh:(q // 2 + 1) * kh, (q % 2) * nh:(q % 2 + 1) * nh]

            m2, m4, m3, m5, m1, m7, m6 = (_dot(operand(aq, LHS[i]), operand(bq, RHS[i])) for i in (1, 3, 2, 4, 0, 6, 5))
            top = [m1 + (m4 - m5) + m7, m3 + m5]
            bottom = [m2 + m4, (m1 - m2) + m3 + m6]
            r = jnp.concatenate([jnp.concatenate(top, axis=1), jnp.concatenate(bottom, axis=1)], axis=0)
            if 2 * kh < k:
                r = r + _dot(a[:, 2 * kh:].astype(BF16), b[2 * kh:, :2 * nh].astype(BF16))
            if 2 * nh < n:
                r = jnp.concatenate([r, _dot(a.astype(BF16), b[:, 2 * nh:].astype(BF16))], axis=1)
            return r

        def combine(quad, spec):
            qa, sign, qb = spec
            if not sign:
                return quad(qa)
            x, y = quad(qa).astype(F32), quad(qb).astype(F32)
            return x + y if sign > 0 else x - y

        OUT = ({0: 1, 3: 1, 4: -1, 6: 1}, {2: 1, 4: 1}, {1: 1, 3: 1}, {0: 1, 1: -1, 2: 1, 5: 1})

        def strassen(prod, emit, order):
            acc, seen = {}, set()
            for i in order:
                m = prod(i)
                seen.add(i)
                for q, terms in enumerate(OUT):
                    if i in terms:
                        if q in acc:
                            sign, v = acc[q]
                            acc[q] = (sign, v + m if sign == terms[i] else v - m) if sign > 0 or terms[i] < 0 else (1, m - v)
                        else:
                            acc[q] = (terms[i], m)
                        if set(terms) <= seen:
                            emit(q, acc[q][1])

        def quadrant(q, n0):
            return pl.ds((q // 2) * DH, DH), pl.ds((q % 2) * SH + n0, SC)

        def out_copy(q, j, n0):
            idx = quadrant(q, n0)
            return pltpu.make_async_copy(out_v.at[idx], out_hbm.at[idx], osems.at[4 * j + q])

        with scope("mlp"):
            norm_block(NB - 1)
            b1f = 0.5 * b1_v[...].astype(F32).reshape(1, F)
            b2f_v[...] = b2_v[...].astype(F32).reshape(1, S)

            def hq(q):
                return hn_v[(q // 2) * DH:(q // 2 + 1) * DH, (q % 2) * SH:(q % 2 + 1) * SH]

            def w1q(q):
                return w1_v[(q // 2) * SH:(q // 2 + 1) * SH, (q % 2) * FH:(q % 2 + 1) * FH]

            def first(i):
                return product(combine(hq, LHS[i]), combine(w1q, RHS[i]), i in DEEP1)

            gq = {}

            def act(q, v):
                gq[q] = _gelu_of_half(v + b1f[:, (q % 2) * FH:(q % 2 + 1) * FH])
                for i, (qa, sign, qb) in enumerate(LHS):
                    need = {qa, qb} if sign else {qa}
                    if q in need and need <= set(gq):
                        g_v[i] = combine(gq.get, LHS[i]).astype(g_v.dtype)

            strassen(first, act, ORD1)

            def mlp2(j, carry):
                n0 = j * SC if isinstance(j, int) else pl.multiple_of(j * SC, SC)

                def w2q(q):
                    return w2_v[(q // 2) * FH:(q // 2 + 1) * FH, pl.ds((q % 2) * SH + n0, SC)]

                def second(i):
                    return product(g_v[i], combine(w2q, RHS[i]), i in DEEP2)

                def finish(q, v):
                    idx = quadrant(q, n0)
                    out_v[idx] = (ht_v[idx] + (v + b2f_v[:, idx[1]])).astype(BF16)
                    if not LATE:
                        out_copy(q, j, n0).start()

                strassen(second, finish, ORD2)
                return carry

        with scope("mlp2"):
            for j in range(NPEEL):
                mlp2(j, 0)
            if NPEEL < SH // SC:
                lax.fori_loop(NPEEL, SH // SC, mlp2, 0)
        with scope("tail"):
            if LATE:
                for j in range(SH // SC):
                    for q in range(4):
                        out_copy(q, j, j * SC).start()
            for j in range(SH // SC):
                for q in range(4):
                    out_copy(q, j, j * SC).wait()

    scratch = [
        pltpu.VMEM((4, D, HG, E), BF16), pltpu.VMEM((2, D, HG, E), BF16), pltpu.VMEM((H, D, E), BF16),
        pltpu.VMEM((2, 2, D * PG, LANE), U32), pltpu.VMEM((2, D * PG, LANE), U32),
        pltpu.VMEM((WB, DM // 2, 2 * LANE), U32), pltpu.VMEM((WB, DM // 2, 2 * LANE), U32),
        pltpu.VMEM((NP // 2, D // 2, 2 * LANE), U32), pltpu.VMEM((NP, HP, DP), U32),
        pltpu.VMEM((D, S), BF16), pltpu.VMEM((S, DP), F32), pltpu.VMEM((S, DP), F32),
        pltpu.VMEM((D, S), F32),
        pltpu.VMEM((S, F), BF16), pltpu.VMEM((F, S), BF16),
        pltpu.VMEM((7, D // 2, F // 2), F32 if GU else BF16), pltpu.VMEM((D, S), F32), pltpu.VMEM((D, S), BF16),
        pltpu.VMEM((M, D), BF16), pltpu.VMEM((F,), BF16), pltpu.VMEM((S,), BF16), pltpu.VMEM((1, S), F32),
        pltpu.SemaphoreType.DMA((7,)), pltpu.SemaphoreType.DMA((4,)), pltpu.SemaphoreType.DMA((NP,)),
        pltpu.SemaphoreType.DMA((2 * NC,)),
        pltpu.SemaphoreType.DMA((2 * S // SC,)),
    ]
    return kernel, scratch


def build(cfg):
    @functools.partial(jax.jit, static_argnames=("A_seg_len",))
    def fn(A_x, A_mem0, A_Wq, A_Wk, A_Wv, A_Wo, A_seg_len, B_x, B_w1, B_b1, B_w2, B_b2):
        del B_x
        _, S, D = A_x.shape
        _, H, E = A_Wq.shape
        M = A_mem0.shape[1]
        F = B_w1.shape[1]
        kernel, scratch = make_kernel(S, D, H, E, M, A_seg_len, F, cfg)
        hbm = pl.BlockSpec(memory_space=pltpu.HBM)
        out = pl.pallas_call(
            kernel,
            out_shape=pltpu.HBM((D, S), A_x.dtype),
            in_specs=[hbm] * 10,
            out_specs=hbm,
            scratch_shapes=scratch,
            compiler_params=pltpu.CompilerParams(vmem_limit_bytes=110 * 1024 * 1024, flags=cfg.get('flags')),
        )(A_x.reshape(S, D).T, A_mem0.reshape(M, D), A_Wq, A_Wk, A_Wv, A_Wo.transpose(0, 2, 1),
          B_w1, B_b1, B_w2, B_b2)
        return out.T.reshape(A_x.shape)

    return fn


pallas_sequential_preLN__memory_aug_recurrent_mem_tr__mixer_token_mlp__prompt_kernel = build({})
```

```python
import functools

import jax
import jax.numpy as jnp
from jax import lax
from jax.experimental import pallas as pl
from jax.experimental.pallas import tpu as pltpu

F32 = jnp.float32
BF16 = jnp.bfloat16
U32 = jnp.uint32
LANE = 128
EPS = 1e-5
LOG2E = 1.4426950408889634
MASKED = -1000000000.0

_dot = functools.partial(lax.dot_general, dimension_numbers=(((1,), (0,)), ((), ())),
                         preferred_element_type=F32)
_dot_nt = functools.partial(lax.dot_general, dimension_numbers=(((1,), (1,)), ((), ())),
                            preferred_element_type=F32)

_LHS = ((0, 1, 3), (2, 1, 3), (0, 0, 0), (3, 0, 0), (0, 1, 1), (2, -1, 0), (1, -1, 3))
_RHS = ((0, 1, 3), (0, 0, 0), (1, -1, 3), (2, -1, 0), (3, 0, 0), (0, 1, 1), (2, 1, 3))
_OUT = ({0: 1, 3: 1, 4: -1, 6: 1}, {2: 1, 4: 1}, {1: 1, 3: 1}, {0: 1, 1: -1, 2: 1, 5: 1})


def _layernorm_t(v, gain=None):
    c = v - jnp.mean(v, axis=0, keepdims=True)
    inv = lax.rsqrt(jnp.mean(c * c, axis=0, keepdims=True) + EPS)
    return c * (inv if gain is None else inv * gain)


def _gelu_of_half(v):
    c = 0.7978845608028654
    return v + v * jnp.tanh(v * (2.0 * c + (8.0 * 0.044715 * c) * (v * v)))


def _lo_f32(w):
    return pltpu.bitcast(w << 16, F32)


def _hi_f32(w):
    return pltpu.bitcast(w & jnp.uint32(0xFFFF0000), F32)


def _pack(v):
    return pltpu.bitcast(v.astype(BF16), U32)


def _interleave(even, odd):
    return pltpu.bitcast(pltpu.pack_elementwise([even, odd], packed_dtype=BF16), U32)


def _unpack(w):
    return pltpu.bitcast(w, BF16)


def _combine(quad, spec):
    p, sign, q = spec
    if not sign:
        return quad(p)
    x, y = quad(p).astype(F32), quad(q).astype(F32)
    return x + y if sign > 0 else x - y


def _strassen(prod, emit, order):
    acc = {}
    for n, i in enumerate(order):
        m = prod(i)
        for q, terms in enumerate(_OUT):
            if i not in terms:
                continue
            if q not in acc:
                acc[q] = (terms[i], m)
            elif acc[q][0] == terms[i]:
                acc[q] = (terms[i], acc[q][1] + m)
            else:
                acc[q] = (1, acc[q][1] - m if terms[i] < 0 else m - acc[q][1])
            if all(t in order[:n + 1] for t in terms):
                emit(q, acc[q][1])


def _product(a, b, split, strip, order):
    if not split:
        return _dot(a.astype(BF16), b.astype(BF16))
    (m, k), n = a.shape, b.shape[1]
    mh, kh, nh = m // 2, k // (2 * LANE) * LANE, n // (2 * LANE) * LANE
    af, bf = a.astype(F32), b.astype(F32)

    def aq(q):
        return af[(q // 2) * mh:(q // 2 + 1) * mh, (q % 2) * kh:(q % 2 + 1) * kh]

    left = [_combine(aq, spec).astype(BF16) for spec in _LHS]
    quads = [[] for _ in range(4)]
    for c in range(0, nh, strip):
        def bq(q):
            return bf[(q // 2) * kh:(q // 2 + 1) * kh, (q % 2) * nh + c:(q % 2) * nh + c + strip]

        _strassen(lambda i: _dot(left[i], _combine(bq, _RHS[i]).astype(BF16)),
                  lambda q, v: quads[q].append(v), order)
    r = jnp.concatenate([jnp.concatenate(quads[0] + quads[1], axis=1),
                         jnp.concatenate(quads[2] + quads[3], axis=1)], axis=0)
    if 2 * kh < k:
        r = r + _dot(a[:, 2 * kh:].astype(BF16), b[2 * kh:, :2 * nh].astype(BF16))
    if 2 * nh < n:
        r = jnp.concatenate([r, _dot(a.astype(BF16), b[:, 2 * nh:].astype(BF16))], axis=1)
    return r


def _each(n, fn):
    def body(i, carry):
        fn(i)
        return carry

    lax.fori_loop(0, n, body, 0)


def _make_kernel(S, D, H, E, M, L, F):
    DM = (D // LANE) * LANE
    DR = D - DM
    DP = DM + LANE
    NT = DM // LANE
    NP = H // 2
    HG = H // 2
    PG = HG // 2
    R = M + L
    KT = H * R // LANE
    WB = NT * NP + NP // 2
    NB = S // LANE
    SB = LANE // L
    DH, FH, SH = D // 2, F // 2, S // 2
    SC = 2 * LANE
    NJ = SH // SC
    assert (D, H, E, M, R) == (448, 16, 2 * LANE, 8, 40) and S % (2 * SC) == 0 and F % (2 * LANE) == 0

    TILE = ((0, 1, 4), (2, 3, 5), (8, 9, 12), (10, 11, 13), (6, 7, 14))
    LAST = H - 1
    KPAIR = ((2, 0), (3, 1), (5, 4), (7, 6))
    KPOS = {g * HG + j: (g * PG + i, half)
            for g in range(2) for i, pr in enumerate(KPAIR) for half, j in enumerate(pr)}
    K_CHUNKS = ((2 * LANE, D - 2 * LANE), (0, 2 * LANE))

    def kernel(xt_hbm, mem0_hbm, wq_hbm, wk_hbm, wv_hbm, wo_hbm, w1_hbm, b1_hbm, w2_hbm, b2_hbm,
               out_hbm,
               raw, raw_k, wo_v, sw, sk, wu, wz, wt, wb, xt_v, xn, o_v, ht_v, hn_v,
               w1_v, w2_v, g_v, out_v, mem0_v, b1_v, b2_v, b2f_v,
               sems, sem_r, sem_o, sem_k):
        def heads(g):
            return pl.ds(pl.multiple_of(g * HG, HG), HG)

        def tokens(b):
            return pl.ds(b * LANE if isinstance(b, int) else pl.multiple_of(b * LANE, LANE), LANE)

        def cp_v(g):
            return pltpu.make_async_copy(wv_hbm.at[:, heads(g), :], raw.at[g], sem_r.at[g])

        def cp_q(g):
            return pltpu.make_async_copy(wq_hbm.at[:, heads(g), :], raw.at[2 + g], sem_r.at[2 + g])

        def cp_k(g, c):
            rows = pl.ds(*K_CHUNKS[c])
            return pltpu.make_async_copy(wk_hbm.at[rows, heads(g), :], raw_k.at[g, rows], sem_k.at[2 * g + c])

        def cp_o(p):
            return pltpu.make_async_copy(wo_hbm.at[pl.ds(2 * p, 2)], wo_v.at[pl.ds(2 * p, 2)], sem_o.at[p])

        def cp_x(b, sem):
            return pltpu.make_async_copy(xt_hbm.at[:, tokens(b)], xt_v.at[b], sem)

        def cp_w2(j, half):
            return pltpu.make_async_copy(w2_hbm.at[:, pl.ds(half * SH + j * SC, SC)],
                                         w2_v.at[j, :, pl.ds(half * SC, SC)], sems.at[1])

        def cp_out(q, j):
            rows = pl.ds((q // 2) * DH, DH)
            n0 = j * SC if isinstance(j, int) else pl.multiple_of(j * SC, SC)
            return pltpu.make_async_copy(out_v.at[j, rows, pl.ds((q % 2) * SC, SC)],
                                         out_hbm.at[rows, pl.ds((q % 2) * SH + n0, SC)], sems.at[2])

        def start_values(g):
            cp_v(g).start()
            _each(PG, lambda pp: cp_o(g * PG + pp).start())

        def start_keys(g):
            cp_q(g).start()
            _each(len(K_CHUNKS), lambda i: [pl.when(i == c)(cp_k(g, c).start) for c in range(len(K_CHUNKS))])
            pl.when(g == 0)(cp_x(0, sems.at[3]).start)

        _each(2, start_values)
        _each(2, start_keys)
        small = [pltpu.make_async_copy(src, dst, sems.at[0])
                 for src, dst in ((mem0_hbm, mem0_v), (b1_hbm, b1_v), (b2_hbm, b2_v))]
        for cp in small:
            cp.start()
        _each(NB - 1, lambda i: cp_x(i + 1, sems.at[0]).start())
        late = [pltpu.make_async_copy(w1_hbm, w1_v, sems.at[1])]
        late += [cp_w2(j, half) for j in range(NJ) for half in range(2)]
        for cp in late:
            cp.start()

        low = lax.broadcasted_iota(jnp.int32, (1, LANE), 1) < DR
        halves = (_lo_f32, _hi_f32)
        o_v[0:LANE, :] = jnp.zeros((LANE, DP), F32)

        def relayout(src, dst, d0, nd):
            for d in range(d0, d0 + nd, DR):
                u = pltpu.bitcast(src[d:d + DR].reshape(DR * HG, E), U32)
                dst[0, d * PG:(d + DR) * PG, :] = u[:, :LANE]
                dst[1, d * PG:(d + DR) * PG, :] = u[:, LANE:]

        def pair(src, pp, d0, nd, step=1):
            idx = pl.ds(d0 * PG + pp, nd, stride=step * PG)
            return jnp.concatenate([src[0, idx, :], src[1, idx, :]], axis=1)

        def store_main(dst, g, j, d0, w):
            rows = pl.ds(d0 // 2, w.shape[0])
            for t in range(NT):
                dst[t * NP + g * PG + j // 2, rows, (j % 2) * LANE:(j % 2 + 1) * LANE] = w[:, t * LANE:(t + 1) * LANE]

        def store_rem(dst, g, i, d0, w):
            rows = pl.ds(d0 // 2, w.shape[0])
            dst[NT * NP + g * (PG // 2) + i // 2, rows, (i % 2) * LANE:(i % 2 + 1) * LANE] = w

        def fold_values(g):
            rem = {}
            for j in range(HG):
                pp, par = divmod(j, 2)
                p = g * PG + pp
                for i in {0: (0,), 2: (1,), 4: (2, 3)}.get(j, ()):
                    cp_o(g * PG + i).wait()
                if par == 0:
                    words = [pair(sw.at[g], pp, i, DH, 2) for i in range(2)]
                if j == HG - 1:
                    pltpu.make_async_copy(raw.at[g + 1], raw.at[g + 1], sem_r.at[g + 1]).wait()
                even, odd = map(halves[par], words)
                o = wo_v[2 * p + par]

                def edge():
                    rem[j] = _dot_nt(o[DM:], jnp.concatenate([even, odd, odd[:DR]], axis=0).astype(BF16))
                    for i, hs in enumerate(KPAIR):
                        if j == max(hs):
                            tile = jnp.concatenate([rem[h] for h in hs], axis=0).T
                            tile = _interleave(tile[:DH], tile[DH:D])
                            store_rem(wz, g, i, 0, tile[:DM // 2])
                            t0 = tile[DM // 2:]
                            t1 = pltpu.roll(t0, DR, 1)
                            for h, both in zip(hs, (jnp.where(low, t0, t1), jnp.where(low, t1, t0))):
                                wb[g * PG + h // 2, (h % 2) * (DR // 2):(h % 2 + 1) * (DR // 2), DM:] = both

                edge_last = j in (0, 2, 4)
                if not edge_last:
                    edge()
                r = _interleave(_dot_nt(even, o[:DM]), _dot_nt(odd, o[:DM]))
                if j == HG - 1:
                    relayout(raw.at[g + 1], sw.at[1 - g], 0, D)
                store_main(wz, g, j, 0, r[:DM // 2])
                wb[p, par * (DR // 2):(par + 1) * (DR // 2), :DM] = r[DM // 2:]
                if edge_last:
                    edge()

        def norm_input(b):
            xv = _layernorm_t(xt_v[b].astype(F32))
            xn[tokens(b), :] = jnp.concatenate([xv, xv[DM:]], axis=0).T

        def fold_keys(g):
            def fetch(c):
                cp_k(g, c).wait()
                relayout(raw_k.at[g], sk, *K_CHUNKS[c])

            query = {}
            for c, (d0, nd) in enumerate(K_CHUNKS):
                nm = min(nd, DM - d0)
                rem = {}
                for pp in range(PG):
                    if c == 0 and pp == 0:
                        fetch(0)
                    if c == 0 and pp == PG - 1:
                        fetch(1)
                    words = [pair(sk, pp, d0 + i, nm // 2, 2) for i in range(2)]
                    if c == 0:
                        wq = pair(sw.at[g], pp, 0, D)
                        for par, half in enumerate(halves):
                            q = half(wq)
                            query[2 * pp + par] = q[:DM].astype(BF16), q[DM:]
                    tail = []
                    if nm < nd:
                        wr = pair(sk, pp, DM, DR)
                        for par, half in enumerate(halves):
                            qm, qr = query[2 * pp + par]
                            rhs = jnp.concatenate([qm, jnp.concatenate([qr, qr], axis=0).astype(BF16)], axis=0)
                            tail.append(_dot_nt(half(wr), rhs))

                    def edge(par):
                        j = 2 * pp + par
                        k = jnp.concatenate([halves[par](w) for w in words], axis=0)
                        rem[j] = _dot_nt(query[j][1], k.astype(BF16))
                        for i, hs in enumerate(KPAIR):
                            if j == max(hs):
                                tile = jnp.concatenate([rem[h] for h in hs], axis=0).T
                                store_rem(wu, g, i, d0, _interleave(tile[:nm // 2], tile[nm // 2:]))

                    def body(par):
                        j = 2 * pp + par
                        store_main(wu, g, j, d0, _interleave(*(_dot_nt(halves[par](w), query[j][0]) for w in words)))

                    body(0)
                    edge(0)
                    edge(1)
                    body(1)
                    if tail:
                        wt[g * (PG // 2) + pp // 2, :, (pp % 2) * LANE:(pp % 2 + 1) * LANE] = _pack(
                            jnp.concatenate(tail, axis=0).T[:D])

            @pl.when(g == 0)
            def _():
                cp_q(1).wait()
                cp_x(0, sems.at[3]).wait()
                relayout(raw.at[3], sw.at[1], 0, D)
                norm_input(0)

        cp_v(0).wait()
        relayout(raw.at[0], sw.at[0], 0, D)
        _each(2, fold_values)
        _each(2, fold_keys)

        def project(ha, w_ref, t):
            base, n = (t * NP, NP) if t < NT else (NT * NP, NP // 2)
            out = []
            for p0 in range(0, n, 4):
                r = _dot(ha, _unpack(jnp.concatenate([w_ref[base + p0 + i] for i in range(4)], axis=1)))
                out += [r[:, i * LANE:(i + 1) * LANE] for i in range(8)]
            return out

        def main_blocks(ha, w_ref, t):
            hd = project(ha, w_ref, t)
            return [jnp.concatenate([hd[h] for h in TILE[k]] + [hd[LAST][k * M:(k + 1) * M]], axis=0)
                    for k in range(KT)]

        def rem_blocks(ha, w_ref, rr):
            rem = project(ha, w_ref, NT)
            blocks = []
            for k in range(KT):
                own = TILE[k][2] % 2
                mine = low if own == 0 else jnp.logical_not(low)

                def part(h):
                    i, half = KPOS[h]
                    v = rem[i][k * M:(k + 1) * M] if h == LAST else rem[i]
                    if half == own:
                        v = pltpu.roll(v, DR, 1)
                    return jnp.where(mine, rr if h == TILE[k][2] else 0.0, v)

                blocks.append(jnp.concatenate([part(h) for h in TILE[k] + (LAST,)], axis=0))
            return blocks

        scale = float(E) ** -0.5
        key = lax.broadcasted_iota(jnp.int32, (R, 3 * R), 0)
        col = lax.broadcasted_iota(jnp.int32, (R, 3 * R), 1)
        qry = col - jnp.where(col >= R, R, 0) - jnp.where(col >= 2 * R, R, 0)
        grp = lax.broadcasted_iota(jnp.int32, (M, 3 * R), 1)

        def softmax_keys(v):
            v = jnp.where((qry < M) | (qry >= key), v, MASKED / scale)
            e = jnp.exp2((v - jnp.max(v, axis=0, keepdims=True)) * (scale * LOG2E))
            return e * (1.0 / jnp.sum(e, axis=0, keepdims=True))

        def shift(v, n):
            if n == 0:
                return v
            v = jnp.concatenate([v, jnp.zeros((M, LANE - 3 * R), F32)], axis=1)
            return pltpu.roll(v, n % LANE, 1)[:, :3 * R]

        def step(s, mem, side):
            rows = pl.ds(pl.multiple_of(s * L, L), L)
            hh = jnp.concatenate([mem, xn[rows, :]], axis=0)
            ha, rr = hh[:, :DM], hh[:, DM:]
            own = jnp.concatenate([jnp.where(low, rr, 0.0), jnp.where(low, 0.0, rr),
                                   jnp.zeros((LANE - 2 * R, LANE), F32)], axis=0)
            own_t = own.T
            side()

            kb, tq = {}, {}
            for t in (0, NT, 1, 2):
                kb[t] = [b.T for b in (main_blocks(ha, wu, t) if t < NT else rem_blocks(ha, wu, rr))]
            for t in (1, 0):
                r = _dot(hh[:, :D], _unpack(jnp.concatenate([wt[2 * t], wt[2 * t + 1]], axis=1)))
                for i in range(4):
                    tq[4 * t + i] = r[:, i * LANE:(i + 1) * LANE]
            vrem = rem_blocks(ha, wz, rr)
            sc = [None] * (KT + 1)
            for k in (3, 4, KT, 0, 1, 2):
                if k == KT:
                    sc[k] = _dot(tq[LAST // 2], own_t.astype(BF16))
                    continue
                i, half = divmod(TILE[k][2], 2)
                third = jnp.where(low, tq[i], rr) if half == 0 else jnp.where(low, rr, tq[i])
                rhs = jnp.concatenate([jnp.concatenate([kb[t][k] for t in range(NT)], axis=0), kb[NT][k], own_t], axis=0)
                sc[k] = _dot(jnp.concatenate([ha, third, tq[TILE[k][0] // 2]], axis=1), rhs.astype(BF16))
            vb = [main_blocks(ha, wz, t) for t in range(NT)]

            sa = jnp.concatenate(sc[:3], axis=0).T
            sb = jnp.concatenate(sc[3:], axis=0).T
            g1, g3 = grp < R, grp >= 2 * R
            tail = [(sa if k < 3 else sb)[3 * R:] for k in range(KT)]
            home = sb[R:2 * R] + jnp.concatenate(
                [jnp.where(g3, shift(tail[k], (2 - k % 3) * R), 0.0) for k in range(KT)], axis=0)
            ps = [softmax_keys(v) for v in (sa[0:R], sa[R:2 * R], sa[2 * R:3 * R], sb[0:R], home, sb[2 * R:3 * R])]
            back = [shift(ps[4][k * M:(k + 1) * M], (k % 3 - 2) * R) for k in range(KT)]
            ta = jnp.where(g1, back[0], jnp.where(g3, back[2], back[1]))
            tb = jnp.where(g1, back[3], back[4])
            pa = jnp.concatenate(ps[:3] + [ta], axis=0).T
            pb = jnp.concatenate(ps[3:] + [tb], axis=0).T
            pm = [pa[i * R:(i + 1) * R] for i in range(3)] + [pb[i * R:(i + 1) * R] for i in range(2)]

            ra, rb = _dot(pa, own.astype(BF16)), _dot(pb, own.astype(BF16))
            xa = [ra[i * R:(i + 1) * R] for i in range(3)] + [rb[i * R:(i + 1) * R] for i in range(2)]
            xb = [_dot(pm[k], vrem[k].astype(BF16)) for k in range(KT)]
            rhs = jnp.concatenate([jnp.concatenate([vb[t][k] for t in range(NT)], axis=1) for k in range(KT)], axis=0)
            oa = _dot(jnp.concatenate(pm, axis=1), rhs.astype(BF16))
            single = {TILE[k][2]: xb[k] for k in range(KT)}
            single[LAST] = rb[2 * R:]
            both = {TILE[k][0] // 2: xa[k] for k in range(KT)}
            pr = [both[p] if p in both else jnp.where(low, single[2 * p], single[2 * p + 1]) for p in range(NP)]
            ob = _dot(jnp.concatenate(pr, axis=1), _unpack(jnp.concatenate([wb[p] for p in range(NP)], axis=0)))
            hi_sum, lo_sum = (functools.reduce(jnp.add, [xb[k] for k in range(KT) if TILE[k][2] % 2 == half])
                              for half in range(2))
            orem = jnp.where(low, lo_sum, hi_sum)
            o = ob + jnp.concatenate([oa, orem + pltpu.roll(orem, DR, 1)], axis=1)
            o_v[rows, :] = o[M:]
            return o[:M]

        def norm_output(b):
            ht = xt_v[b].astype(F32) + o_v[tokens(b), :].T[:D]
            ht_v[b] = ht
            hn_v[b] = _layernorm_t(_layernorm_t(ht), 0.5)

        def block(b, mem):
            def side():
                norm_output(jnp.maximum(b - 1, 0))
                norm_input(jnp.minimum(b + 1, NB - 1))

            for j in range(SB):
                mem = step(b * SB + j, mem, side if j == 1 else lambda: None)
            return mem

        for cp in small:
            cp.wait()
        _each(NB - 1, lambda i: cp_x(i + 1, sems.at[0]).wait())
        m0 = mem0_v[...].astype(F32)
        lax.fori_loop(0, NB, block, jnp.concatenate([m0, m0[:, DM:]], axis=1))
        for cp in late:
            cp.wait()

        norm_output(NB - 1)
        b1f = 0.5 * b1_v[...].astype(F32).reshape(1, F)
        b2f = b2_v[...].astype(F32).reshape(1, S)
        for i in range(NB):
            b2f_v[i] = b2f[:, i * LANE:(i + 1) * LANE]

        def hq(q):
            return jnp.concatenate([hn_v[(q % 2) * (NB // 2) + i, (q // 2) * DH:(q // 2 + 1) * DH, :]
                                    for i in range(NB // 2)], axis=1)

        def w1q(q):
            return w1_v[(q // 2) * SH:(q // 2 + 1) * SH, (q % 2) * FH:(q % 2 + 1) * FH]

        gq = {}

        def activate(q, v):
            gq[q] = _gelu_of_half(v + b1f[:, (q % 2) * FH:(q % 2 + 1) * FH])
            for i, (qa, sign, qb) in enumerate(_LHS):
                need = (qa, qb) if sign else (qa,)
                if q in need and all(n in gq for n in need):
                    g_v[i] = _combine(gq.get, _LHS[i])

        _strassen(lambda i: _product(_combine(hq, _LHS[i]), _combine(w1q, _RHS[i]), i in (1, 3, 4),
                                     LANE, (1, 3, 4, 2, 0, 5, 6)),
                  activate, (2, 5, 4, 1, 3, 0, 6))

        def mlp2(j):
            def w2q(q):
                return w2_v[j, (q // 2) * FH:(q // 2 + 1) * FH, (q % 2) * SC:(q % 2 + 1) * SC]

            def finish(q, v):
                rows = slice((q // 2) * DH, (q // 2 + 1) * DH)
                first = (q % 2) * (NB // 2) + j * (SC // LANE)
                ht = jnp.concatenate([ht_v[first + i, rows, :] + b2f_v[first + i] for i in range(SC // LANE)], axis=1)
                out_v[j, rows, (q % 2) * SC:(q % 2 + 1) * SC] = (ht + v).astype(BF16)
                cp_out(q, j).start()

            _strassen(lambda i: _product(g_v[i], _combine(w2q, _RHS[i]), i != 0, LANE, (1, 3, 2, 4, 0, 6, 5)),
                      finish, (1, 3, 4, 2, 0, 5, 6))

        _each(NJ, mlp2)
        for j in range(NJ):
            for q in range(4):
                cp_out(q, j).wait()

    words = D * PG + 32
    scratch = [
        pltpu.VMEM((4, D, HG, E), BF16), pltpu.VMEM((2, D, HG, E), BF16), pltpu.VMEM((H, D, E), BF16),
        pltpu.VMEM((2, 2, words, LANE), U32), pltpu.VMEM((2, words, LANE), U32),
        pltpu.VMEM((WB, DM // 2, 2 * LANE), U32), pltpu.VMEM((WB, DM // 2, 2 * LANE), U32),
        pltpu.VMEM((NP // 2, DH, 2 * LANE), U32), pltpu.VMEM((NP, LANE // 2, DP), U32),
        pltpu.VMEM((NB, D, LANE), BF16), pltpu.VMEM((S, DP), F32), pltpu.VMEM((S, DP), F32),
        pltpu.VMEM((NB, D, LANE), F32), pltpu.VMEM((NB, D, LANE), F32),
        pltpu.VMEM((S, F), BF16), pltpu.VMEM((NJ, F, 2 * SC), BF16),
        pltpu.VMEM((7, DH, FH), F32), pltpu.VMEM((NJ, D, 2 * SC), BF16),
        pltpu.VMEM((M, D), BF16), pltpu.VMEM((F,), BF16), pltpu.VMEM((S,), BF16), pltpu.VMEM((NB, 1, LANE), F32),
        pltpu.SemaphoreType.DMA((4,)), pltpu.SemaphoreType.DMA((4,)), pltpu.SemaphoreType.DMA((NP,)),
        pltpu.SemaphoreType.DMA((4,)),
    ]
    return kernel, scratch


@functools.partial(jax.jit, static_argnames=("A_seg_len",))
def pallas_sequential_preLN__memory_aug_recurrent_mem_tr__mixer_token_mlp__prompt_kernel(
        A_x, A_mem0, A_Wq, A_Wk, A_Wv, A_Wo, A_seg_len, B_x, B_w1, B_b1, B_w2, B_b2):
    del B_x
    _, S, D = A_x.shape
    _, H, E = A_Wq.shape
    M = A_mem0.shape[1]
    F = B_w1.shape[1]
    kernel, scratch = _make_kernel(S, D, H, E, M, A_seg_len, F)
    hbm = pl.BlockSpec(memory_space=pltpu.HBM)
    out = pl.pallas_call(
        kernel,
        out_shape=pltpu.HBM((D, S), A_x.dtype),
        in_specs=[hbm] * 10,
        out_specs=hbm,
        scratch_shapes=scratch,
        compiler_params=pltpu.CompilerParams(vmem_limit_bytes=110 * 1024 * 1024),
    )(A_x.reshape(S, D).T, A_mem0.reshape(M, D), A_Wq, A_Wk, A_Wv, A_Wo.transpose(0, 2, 1),
      B_w1, B_b1, B_w2, B_b2)
    return out.T.reshape(A_x.shape)
```

```python
import functools

import jax
import jax.numpy as jnp
from jax import lax
from jax.experimental import pallas as pl
from jax.experimental.pallas import tpu as pltpu

F32 = jnp.float32
BF16 = jnp.bfloat16
U32 = jnp.uint32
LANE = 128
EPS = 1e-5
LOG2E = 1.4426950408889634
MASKED = -1000000000.0

_dot = functools.partial(lax.dot_general, dimension_numbers=(((1,), (0,)), ((), ())),
                         preferred_element_type=F32)
_dot_nt = functools.partial(lax.dot_general, dimension_numbers=(((1,), (1,)), ((), ())),
                            preferred_element_type=F32)

_LHS = ((0, 1, 3), (2, 1, 3), (0, 0, 0), (3, 0, 0), (0, 1, 1), (2, -1, 0), (1, -1, 3))
_RHS = ((0, 1, 3), (0, 0, 0), (1, -1, 3), (2, -1, 0), (3, 0, 0), (0, 1, 1), (2, 1, 3))
_OUT = ({0: 1, 3: 1, 4: -1, 6: 1}, {2: 1, 4: 1}, {1: 1, 3: 1}, {0: 1, 1: -1, 2: 1, 5: 1})


def _layernorm_t(v, gain=None):
    c = v - jnp.mean(v, axis=0, keepdims=True)
    inv = lax.rsqrt(jnp.mean(c * c, axis=0, keepdims=True) + EPS)
    return c * (inv if gain is None else inv * gain)


def _gelu_of_half(v):
    c = 0.7978845608028654
    return v + v * jnp.tanh(v * (2.0 * c + (8.0 * 0.044715 * c) * (v * v)))


def _lo_f32(w):
    return pltpu.bitcast(w << 16, F32)


def _hi_f32(w):
    return pltpu.bitcast(w & jnp.uint32(0xFFFF0000), F32)


def _pack(v):
    return pltpu.bitcast(v.astype(BF16), U32)


def _interleave(even, odd):
    lo, hi = (pltpu.bitcast(v.astype(BF16).astype(F32), U32) for v in (even, odd))
    return (lo >> 16) | hi


def _unpack(w):
    return pltpu.bitcast(w, BF16)


def _combine(quad, spec):
    p, sign, q = spec
    if not sign:
        return quad(p)
    x, y = quad(p).astype(F32), quad(q).astype(F32)
    return x + y if sign > 0 else x - y


def _strassen(prod, emit, order):
    acc = {}
    for n, i in enumerate(order):
        m = prod(i)
        for q, terms in enumerate(_OUT):
            if i not in terms:
                continue
            if q not in acc:
                acc[q] = (terms[i], m)
            elif acc[q][0] == terms[i]:
                acc[q] = (terms[i], acc[q][1] + m)
            else:
                acc[q] = (1, acc[q][1] - m if terms[i] < 0 else m - acc[q][1])
            if all(t in order[:n + 1] for t in terms):
                emit(q, acc[q][1])


def _product(a, b, split, strip, order):
    if not split:
        return _dot(a.astype(BF16), b.astype(BF16))
    (m, k), n = a.shape, b.shape[1]
    mh, kh, nh = m // 2, k // (2 * LANE) * LANE, n // (2 * LANE) * LANE
    af, bf = a.astype(F32), b.astype(F32)

    def aq(q):
        return af[(q // 2) * mh:(q // 2 + 1) * mh, (q % 2) * kh:(q % 2 + 1) * kh]

    left = [_combine(aq, spec).astype(BF16) for spec in _LHS]
    quads = [[] for _ in range(4)]
    for c in range(0, nh, strip):
        def bq(q):
            return bf[(q // 2) * kh:(q // 2 + 1) * kh, (q % 2) * nh + c:(q % 2) * nh + c + strip]

        _strassen(lambda i: _dot(left[i], _combine(bq, _RHS[i]).astype(BF16)),
                  lambda q, v: quads[q].append(v), order)
    r = jnp.concatenate([jnp.concatenate(quads[0] + quads[1], axis=1),
                         jnp.concatenate(quads[2] + quads[3], axis=1)], axis=0)
    if 2 * kh < k:
        r = r + _dot(a[:, 2 * kh:].astype(BF16), b[2 * kh:, :2 * nh].astype(BF16))
    if 2 * nh < n:
        r = jnp.concatenate([r, _dot(a.astype(BF16), b[:, 2 * nh:].astype(BF16))], axis=1)
    return r


def _each(n, fn):
    def body(i, carry):
        fn(i)
        return carry

    lax.fori_loop(0, n, body, 0)


def _make_kernel(S, D, H, E, M, L, F):
    DM = (D // LANE) * LANE
    DR = D - DM
    DP = DM + LANE
    NT = DM // LANE
    NP = H // 2
    HG = H // 2
    PG = HG // 2
    R = M + L
    KT = H * R // LANE
    WB = NT * NP + NP // 2
    NB = S // LANE
    SB = LANE // L
    DH, FH, SH = D // 2, F // 2, S // 2
    SC = 2 * LANE
    NJ = SH // SC
    assert (D, H, E, M, R) == (448, 16, 2 * LANE, 8, 40) and S % (4 * SC) == 0 and F % (2 * LANE) == 0

    TILE = ((0, 1, 4), (2, 3, 5), (8, 9, 12), (10, 11, 13), (6, 7, 14))
    LAST = H - 1
    KPAIR = ((2, 0), (3, 1), (5, 4), (7, 6))
    KPOS = {g * HG + j: (g * PG + i, half)
            for g in range(2) for i, pr in enumerate(KPAIR) for half, j in enumerate(pr)}
    K_CHUNKS = ((2 * LANE, D - 2 * LANE), (0, 2 * LANE))

    def kernel(xt_hbm, mem0_hbm, wq_hbm, wk_hbm, wv_hbm, wo_hbm, w1_hbm, b1_hbm, w2_hbm, b2_hbm,
               out_hbm,
               raw, raw_k, wo_v, sw, sk, wu, wz, wt, wb, xt_v, xn, o_v, ht_v, hn_v,
               w1_v, w2_v, g_v, out_v, mem0_v, b1_v, b2_v, b2f_v,
               sems, sem_r, sem_o, sem_k):
        def heads(g):
            return pl.ds(pl.multiple_of(g * HG, HG), HG)

        def tokens(b):
            return pl.ds(b * LANE if isinstance(b, int) else pl.multiple_of(b * LANE, LANE), LANE)

        def cp_v(g):
            return pltpu.make_async_copy(wv_hbm.at[:, heads(g), :], raw.at[g], sem_r.at[g])

        def cp_q(g):
            return pltpu.make_async_copy(wq_hbm.at[:, heads(g), :], raw.at[2 + g], sem_r.at[2 + g])

        def cp_k(g, c):
            rows = pl.ds(*K_CHUNKS[c])
            return pltpu.make_async_copy(wk_hbm.at[rows, heads(g), :], raw_k.at[g, rows], sem_k.at[2 * g + c])

        def cp_o(p):
            return pltpu.make_async_copy(wo_hbm.at[pl.ds(2 * p, 2)], wo_v.at[pl.ds(2 * p, 2)], sem_o.at[p])

        def cp_x(b, sem):
            return pltpu.make_async_copy(xt_hbm.at[:, tokens(b)], xt_v.at[b], sem)

        def cp_w2(j, half):
            return pltpu.make_async_copy(w2_hbm.at[:, pl.ds(half * SH + j * SC, SC)],
                                         w2_v.at[j, :, pl.ds(half * SC, SC)], sems.at[1])

        def cp_out(q, j):
            rows = pl.ds((q // 2) * DH, DH)
            n0 = j * SC if isinstance(j, int) else pl.multiple_of(j * SC, SC)
            return pltpu.make_async_copy(out_v.at[j, rows, pl.ds((q % 2) * SC, SC)],
                                         out_hbm.at[rows, pl.ds((q % 2) * SH + n0, SC)], sems.at[2])

        def wait_filled(buf, sem):
            pltpu.make_async_copy(buf, buf, sem).wait()

        def start_values(g):
            cp_v(g).start()
            _each(PG, lambda pp: cp_o(g * PG + pp).start())

        def start_keys(g):
            cp_q(g).start()
            _each(len(K_CHUNKS), lambda i: [pl.when(i == c)(cp_k(g, c).start) for c in range(len(K_CHUNKS))])
            pl.when(g == 0)(cp_x(0, sems.at[3]).start)

        _each(2, start_values)
        _each(2, start_keys)
        small = [pltpu.make_async_copy(src, dst, sems.at[0])
                 for src, dst in ((mem0_hbm, mem0_v), (b1_hbm, b1_v), (b2_hbm, b2_v))]
        for cp in small:
            cp.start()
        _each(NB - 1, lambda i: cp_x(i + 1, sems.at[0]).start())
        cp_w1 = pltpu.make_async_copy(w1_hbm, w1_v, sems.at[1])
        cp_w1.start()
        for j in range(NJ):
            for half in range(2):
                cp_w2(j, half).start()

        low = lax.broadcasted_iota(jnp.int32, (1, LANE), 1) < DR
        halves = (_lo_f32, _hi_f32)
        o_v[0:LANE, :] = jnp.zeros((LANE, DP), F32)

        def relayout(src, dst, d0, nd):
            for d in range(d0, d0 + nd, DR):
                u = pltpu.bitcast(src[d:d + DR].reshape(DR * HG, E), U32)
                dst[0, d * PG:(d + DR) * PG, :] = u[:, :LANE]
                dst[1, d * PG:(d + DR) * PG, :] = u[:, LANE:]

        def pair(src, pp, d0, nd, step=1):
            idx = pl.ds(d0 * PG + pp, nd, stride=step * PG)
            return jnp.concatenate([src[0, idx, :], src[1, idx, :]], axis=1)

        def store_main(dst, g, j, d0, w):
            rows = pl.ds(d0 // 2, w.shape[0])
            for t in range(NT):
                dst[t * NP + g * PG + j // 2, rows, (j % 2) * LANE:(j % 2 + 1) * LANE] = w[:, t * LANE:(t + 1) * LANE]

        def store_rem(dst, g, i, d0, w):
            rows = pl.ds(d0 // 2, w.shape[0])
            dst[NT * NP + g * (PG // 2) + i // 2, rows, (i % 2) * LANE:(i % 2 + 1) * LANE] = w

        def fold_values(g):
            rem = {}
            for j in range(HG):
                pp, par = divmod(j, 2)
                p = g * PG + pp
                for i in {0: (0,), 2: (1,), 4: (2, 3)}.get(j, ()):
                    cp_o(g * PG + i).wait()
                if par == 0:
                    words = [pair(sw.at[g], pp, i, DH, 2) for i in range(2)]
                if j == HG - 1:
                    wait_filled(raw.at[g + 1], sem_r.at[g + 1])
                even, odd = map(halves[par], words)
                o = wo_v[2 * p + par]

                def edge():
                    rem[j] = _dot_nt(o[DM:], jnp.concatenate([even, odd, odd[:DR]], axis=0).astype(BF16))
                    for i, hs in enumerate(KPAIR):
                        if j == max(hs):
                            tile = jnp.concatenate([rem[h] for h in hs], axis=0).T
                            tile = _interleave(tile[:DH], tile[DH:D])
                            store_rem(wz, g, i, 0, tile[:DM // 2])
                            t0 = tile[DM // 2:]
                            t1 = pltpu.roll(t0, DR, 1)
                            for h, both in zip(hs, (jnp.where(low, t0, t1), jnp.where(low, t1, t0))):
                                wb[g * PG + h // 2, (h % 2) * (DR // 2):(h % 2 + 1) * (DR // 2), DM:] = both

                edge_last = j in (0, 2, 4)
                if not edge_last:
                    edge()
                r = _interleave(_dot_nt(even, o[:DM]), _dot_nt(odd, o[:DM]))
                if j == HG - 1:
                    relayout(raw.at[g + 1], sw.at[1 - g], 0, D)
                store_main(wz, g, j, 0, r[:DM // 2])
                wb[p, par * (DR // 2):(par + 1) * (DR // 2), :DM] = r[DM // 2:]
                if edge_last:
                    edge()

        def norm_input(b):
            xv = _layernorm_t(xt_v[b].astype(F32))
            xn[tokens(b), :] = jnp.concatenate([xv, xv[DM:]], axis=0).T

        def fold_keys(g):
            def fetch(c):
                cp_k(g, c).wait()
                relayout(raw_k.at[g], sk, *K_CHUNKS[c])

            query = {}
            for c, (d0, nd) in enumerate(K_CHUNKS):
                nm = min(nd, DM - d0)
                rem = {}
                for pp in range(PG):
                    if c == 0 and pp == 0:
                        fetch(0)
                    if c == 0 and pp == PG - 1:
                        fetch(1)
                    words = [pair(sk, pp, d0 + i, nm // 2, 2) for i in range(2)]
                    if c == 0:
                        wq = pair(sw.at[g], pp, 0, D)
                        for par, half in enumerate(halves):
                            q = half(wq)
                            query[2 * pp + par] = q[:DM].astype(BF16), q[DM:]
                    tail = []
                    if nm < nd:
                        wr = pair(sk, pp, DM, DR)
                        for par, half in enumerate(halves):
                            qm, qr = query[2 * pp + par]
                            rhs = jnp.concatenate([qm, jnp.concatenate([qr, qr], axis=0).astype(BF16)], axis=0)
                            tail.append(_dot_nt(half(wr), rhs))

                    def edge(par):
                        j = 2 * pp + par
                        k = jnp.concatenate([halves[par](w) for w in words], axis=0)
                        rem[j] = _dot_nt(query[j][1], k.astype(BF16))
                        for i, hs in enumerate(KPAIR):
                            if j == max(hs):
                                tile = jnp.concatenate([rem[h] for h in hs], axis=0).T
                                store_rem(wu, g, i, d0, _interleave(tile[:nm // 2], tile[nm // 2:]))

                    def body(par):
                        j = 2 * pp + par
                        store_main(wu, g, j, d0, _interleave(*(_dot_nt(halves[par](w), query[j][0]) for w in words)))

                    body(0)
                    edge(0)
                    edge(1)
                    body(1)
                    if tail:
                        wt[g * (PG // 2) + pp // 2, :, (pp % 2) * LANE:(pp % 2 + 1) * LANE] = _pack(
                            jnp.concatenate(tail, axis=0).T[:D])

            @pl.when(g == 0)
            def _():
                cp_q(1).wait()
                cp_x(0, sems.at[3]).wait()
                relayout(raw.at[3], sw.at[1], 0, D)
                norm_input(0)

        cp_v(0).wait()
        relayout(raw.at[0], sw.at[0], 0, D)
        _each(2, fold_values)
        _each(2, fold_keys)

        def project(ha, w_ref, t):
            base, n = (t * NP, NP) if t < NT else (NT * NP, NP // 2)
            out = []
            for p0 in range(0, n, 4):
                r = _dot(ha, _unpack(jnp.concatenate([w_ref[base + p0 + i] for i in range(4)], axis=1)))
                out += [r[:, i * LANE:(i + 1) * LANE] for i in range(8)]
            return out

        def main_blocks(ha, w_ref, t):
            hd = project(ha, w_ref, t)
            return [jnp.concatenate([hd[h] for h in TILE[k]] + [hd[LAST][k * M:(k + 1) * M]], axis=0)
                    for k in range(KT)]

        def rem_blocks(ha, w_ref, rr):
            rem = project(ha, w_ref, NT)
            blocks = []
            for k in range(KT):
                own = TILE[k][2] % 2
                mine = low if own == 0 else jnp.logical_not(low)

                def part(h):
                    i, half = KPOS[h]
                    v = rem[i][k * M:(k + 1) * M] if h == LAST else rem[i]
                    if half == own:
                        v = pltpu.roll(v, DR, 1)
                    return jnp.where(mine, rr if h == TILE[k][2] else 0.0, v)

                blocks.append(jnp.concatenate([part(h) for h in TILE[k] + (LAST,)], axis=0))
            return blocks

        scale = float(E) ** -0.5
        key = lax.broadcasted_iota(jnp.int32, (R, 3 * R), 0)
        col = lax.broadcasted_iota(jnp.int32, (R, 3 * R), 1)
        qry = col - jnp.where(col >= R, R, 0) - jnp.where(col >= 2 * R, R, 0)
        grp = lax.broadcasted_iota(jnp.int32, (M, 3 * R), 1)

        def softmax_keys(v):
            v = jnp.where((qry < M) | (qry >= key), v, MASKED / scale)
            e = jnp.exp2((v - jnp.max(v, axis=0, keepdims=True)) * (scale * LOG2E))
            return e * (1.0 / jnp.sum(e, axis=0, keepdims=True))

        def shift(v, n):
            if n == 0:
                return v
            v = jnp.concatenate([v, jnp.zeros((M, LANE - 3 * R), F32)], axis=1)
            return pltpu.roll(v, n % LANE, 1)[:, :3 * R]

        def step(s, mem, side):
            rows = pl.ds(pl.multiple_of(s * L, L), L)
            hh = jnp.concatenate([mem, xn[rows, :]], axis=0)
            ha, rr = hh[:, :DM], hh[:, DM:]
            own = jnp.concatenate([jnp.where(low, rr, 0.0), jnp.where(low, 0.0, rr),
                                   jnp.zeros((LANE - 2 * R, LANE), F32)], axis=0)
            own_t = own.T
            side()

            kb, tq = {}, {}
            for t in (0, NT, 1, 2):
                kb[t] = [b.T for b in (main_blocks(ha, wu, t) if t < NT else rem_blocks(ha, wu, rr))]
            for t in (1, 0):
                r = _dot(hh[:, :D], _unpack(jnp.concatenate([wt[2 * t], wt[2 * t + 1]], axis=1)))
                for i in range(4):
                    tq[4 * t + i] = r[:, i * LANE:(i + 1) * LANE]
            vrem = rem_blocks(ha, wz, rr)
            sc = [None] * (KT + 1)
            for k in (3, 4, KT, 0, 1, 2):
                if k == KT:
                    sc[k] = _dot(tq[LAST // 2], own_t.astype(BF16))
                    continue
                i, half = divmod(TILE[k][2], 2)
                third = jnp.where(low, tq[i], rr) if half == 0 else jnp.where(low, rr, tq[i])
                rhs = jnp.concatenate([jnp.concatenate([kb[t][k] for t in range(NT)], axis=0), kb[NT][k], own_t], axis=0)
                sc[k] = _dot(jnp.concatenate([ha, third, tq[TILE[k][0] // 2]], axis=1), rhs.astype(BF16))
            vb = [main_blocks(ha, wz, t) for t in range(NT)]

            sa = jnp.concatenate(sc[:3], axis=0).T
            sb = jnp.concatenate(sc[3:], axis=0).T
            g1, g3 = grp < R, grp >= 2 * R
            tail = [(sa if k < 3 else sb)[3 * R:] for k in range(KT)]
            home = sb[R:2 * R] + jnp.concatenate(
                [jnp.where(g3, shift(tail[k], (2 - k % 3) * R), 0.0) for k in range(KT)], axis=0)
            ps = [softmax_keys(v) for v in (sa[0:R], sa[R:2 * R], sa[2 * R:3 * R], sb[0:R], home, sb[2 * R:3 * R])]
            back = [shift(ps[4][k * M:(k + 1) * M], (k % 3 - 2) * R) for k in range(KT)]
            ta = jnp.where(g1, back[0], jnp.where(g3, back[2], back[1]))
            tb = jnp.where(g1, back[3], back[4])
            pa = jnp.concatenate(ps[:3] + [ta], axis=0).T
            pb = jnp.concatenate(ps[3:] + [tb], axis=0).T
            pm = [pa[i * R:(i + 1) * R] for i in range(3)] + [pb[i * R:(i + 1) * R] for i in range(2)]

            ra, rb = _dot(pa, own.astype(BF16)), _dot(pb, own.astype(BF16))
            xa = [ra[i * R:(i + 1) * R] for i in range(3)] + [rb[i * R:(i + 1) * R] for i in range(2)]
            xb = [_dot(pm[k], vrem[k].astype(BF16)) for k in range(KT)]
            rhs = jnp.concatenate([jnp.concatenate([vb[t][k] for t in range(NT)], axis=1) for k in range(KT)], axis=0)
            oa = _dot(jnp.concatenate(pm, axis=1), rhs.astype(BF16))
            single = {TILE[k][2]: xb[k] for k in range(KT)}
            single[LAST] = rb[2 * R:]
            both = {TILE[k][0] // 2: xa[k] for k in range(KT)}
            pr = [both[p] if p in both else jnp.where(low, single[2 * p], single[2 * p + 1]) for p in range(NP)]
            ob = _dot(jnp.concatenate(pr, axis=1), _unpack(jnp.concatenate([wb[p] for p in range(NP)], axis=0)))
            hi_sum, lo_sum = (functools.reduce(jnp.add, [xb[k] for k in range(KT) if TILE[k][2] % 2 == half])
                              for half in range(2))
            orem = jnp.where(low, lo_sum, hi_sum)
            o = ob + jnp.concatenate([oa, orem + pltpu.roll(orem, DR, 1)], axis=1)
            o_v[rows, :] = o[M:]
            return o[:M]

        def norm_output(b):
            ht = xt_v[b].astype(F32) + o_v[tokens(b), :].T[:D]
            ht_v[b] = ht
            hn_v[b] = _layernorm_t(_layernorm_t(ht), 0.5)

        def block(b, mem):
            def side():
                norm_output(jnp.maximum(b - 1, 0))
                norm_input(jnp.minimum(b + 1, NB - 1))

            for j in range(SB):
                mem = step(b * SB + j, mem, side if j == 1 else lambda: None)
            return mem

        for cp in small:
            cp.wait()
        wait_filled(xt_v.at[pl.ds(1, NB - 1)], sems.at[0])
        m0 = mem0_v[...].astype(F32)
        lax.fori_loop(0, NB, block, jnp.concatenate([m0, m0[:, DM:]], axis=1))
        cp_w1.wait()
        wait_filled(w2_v, sems.at[1])

        norm_output(NB - 1)
        b1f = 0.5 * b1_v[...].astype(F32).reshape(1, F)
        b2f = b2_v[...].astype(F32).reshape(1, S)
        for i in range(NB):
            b2f_v[i] = b2f[:, i * LANE:(i + 1) * LANE]

        def hq(q):
            return jnp.concatenate([hn_v[(q % 2) * (NB // 2) + i, (q // 2) * DH:(q // 2 + 1) * DH, :]
                                    for i in range(NB // 2)], axis=1)

        def w1q(q):
            return w1_v[(q // 2) * SH:(q // 2 + 1) * SH, (q % 2) * FH:(q % 2 + 1) * FH]

        gq = {}

        def activate(q, v):
            gq[q] = _gelu_of_half(v + b1f[:, (q % 2) * FH:(q % 2 + 1) * FH])
            for i, (qa, sign, qb) in enumerate(_LHS):
                need = (qa, qb) if sign else (qa,)
                if q in need and all(n in gq for n in need):
                    g_v[i] = _combine(gq.get, _LHS[i])

        _strassen(lambda i: _product(_combine(hq, _LHS[i]), _combine(w1q, _RHS[i]), i in (1, 3, 4),
                                     LANE, (1, 3, 4, 2, 0, 5, 6)),
                  activate, (2, 5, 4, 1, 3, 0, 6))

        def mlp2(j):
            def w2q(q):
                return w2_v[j, (q // 2) * FH:(q // 2 + 1) * FH, (q % 2) * SC:(q % 2 + 1) * SC]

            def finish(q, v):
                rows = slice((q // 2) * DH, (q // 2 + 1) * DH)
                first = (q % 2) * (NB // 2) + j * (SC // LANE)
                ht = jnp.concatenate([ht_v[first + i, rows, :] + b2f_v[first + i] for i in range(SC // LANE)], axis=1)
                out_v[j, rows, (q % 2) * SC:(q % 2 + 1) * SC] = (ht + v).astype(BF16)
                cp_out(q, j).start()

            _strassen(lambda i: _product(g_v[i], _combine(w2q, _RHS[i]), i != 0, LANE, (1, 3, 2, 4, 0, 6, 5)),
                      finish, (1, 3, 4, 2, 0, 5, 6))

        _each(NJ // 2, lambda t: [mlp2(2 * t + n) for n in range(2)])
        for j in range(NJ):
            for q in range(4):
                cp_out(q, j).wait()

    words = D * PG + 32
    scratch = [
        pltpu.VMEM((4, D, HG, E), BF16), pltpu.VMEM((2, D, HG, E), BF16), pltpu.VMEM((H, D, E), BF16),
        pltpu.VMEM((2, 2, words, LANE), U32), pltpu.VMEM((2, words, LANE), U32),
        pltpu.VMEM((WB, DM // 2, 2 * LANE), U32), pltpu.VMEM((WB, DM // 2, 2 * LANE), U32),
        pltpu.VMEM((NP // 2, DH, 2 * LANE), U32), pltpu.VMEM((NP, LANE // 2, DP), U32),
        pltpu.VMEM((NB, D, LANE), BF16), pltpu.VMEM((S, DP), F32), pltpu.VMEM((S, DP), F32),
        pltpu.VMEM((NB, D, LANE), F32), pltpu.VMEM((NB, D, LANE), F32),
        pltpu.VMEM((S, F), BF16), pltpu.VMEM((NJ, F, 2 * SC), BF16),
        pltpu.VMEM((7, DH, FH), F32), pltpu.VMEM((NJ, D, 2 * SC), BF16),
        pltpu.VMEM((M, D), BF16), pltpu.VMEM((F,), BF16), pltpu.VMEM((S,), BF16), pltpu.VMEM((NB, 1, LANE), F32),
        pltpu.SemaphoreType.DMA((4,)), pltpu.SemaphoreType.DMA((4,)), pltpu.SemaphoreType.DMA((NP,)),
        pltpu.SemaphoreType.DMA((4,)),
    ]
    return kernel, scratch


@functools.partial(jax.jit, static_argnames=("A_seg_len",))
def pallas_sequential_preLN__memory_aug_recurrent_mem_tr__mixer_token_mlp__prompt_kernel(
        A_x, A_mem0, A_Wq, A_Wk, A_Wv, A_Wo, A_seg_len, B_x, B_w1, B_b1, B_w2, B_b2):
    del B_x
    _, S, D = A_x.shape
    _, H, E = A_Wq.shape
    M = A_mem0.shape[1]
    F = B_w1.shape[1]
    kernel, scratch = _make_kernel(S, D, H, E, M, A_seg_len, F)
    hbm = pl.BlockSpec(memory_space=pltpu.HBM)
    out = pl.pallas_call(
        kernel,
        out_shape=pltpu.HBM((D, S), A_x.dtype),
        in_specs=[hbm] * 10,
        out_specs=hbm,
        scratch_shapes=scratch,
        compiler_params=pltpu.CompilerParams(vmem_limit_bytes=110 * 1024 * 1024),
    )(A_x.reshape(S, D).T, A_mem0.reshape(M, D), A_Wq, A_Wk, A_Wv, A_Wo.transpose(0, 2, 1),
      B_w1, B_b1, B_w2, B_b2)
    return out.T.reshape(A_x.shape)
```

```python
import functools

import jax
import jax.numpy as jnp
from jax import lax
from jax.experimental import pallas as pl
from jax.experimental.pallas import tpu as pltpu

F32 = jnp.float32
BF16 = jnp.bfloat16
U32 = jnp.uint32
LANE = 128
EPS = 1e-5
LOG2E = 1.4426950408889634
MASKED = -1000000000.0

_dot = functools.partial(lax.dot_general, dimension_numbers=(((1,), (0,)), ((), ())),
                         preferred_element_type=F32)
_dot_nt = functools.partial(lax.dot_general, dimension_numbers=(((1,), (1,)), ((), ())),
                            preferred_element_type=F32)

_LHS = ((0, 1, 3), (2, 1, 3), (0, 0, 0), (3, 0, 0), (0, 1, 1), (2, -1, 0), (1, -1, 3))
_RHS = ((0, 1, 3), (0, 0, 0), (1, -1, 3), (2, -1, 0), (3, 0, 0), (0, 1, 1), (2, 1, 3))
_OUT = ({0: 1, 3: 1, 4: -1, 6: 1}, {2: 1, 4: 1}, {1: 1, 3: 1}, {0: 1, 1: -1, 2: 1, 5: 1})


def _layernorm_t(v, gain=None):
    c = v - jnp.mean(v, axis=0, keepdims=True)
    inv = lax.rsqrt(jnp.mean(c * c, axis=0, keepdims=True) + EPS)
    return c * (inv if gain is None else inv * gain)


def _gelu_of_half(v):
    c = 0.7978845608028654
    return v + v * jnp.tanh(v * (2.0 * c + (8.0 * 0.044715 * c) * (v * v)))


def _lo_f32(w):
    return pltpu.bitcast(w << 16, F32)


def _hi_f32(w):
    return pltpu.bitcast(w & jnp.uint32(0xFFFF0000), F32)


def _pack(v):
    return pltpu.bitcast(v.astype(BF16), U32)


def _interleave(even, odd):
    lo, hi = (pltpu.bitcast(v.astype(BF16).astype(F32), U32) for v in (even, odd))
    return (lo >> 16) | hi


def _unpack(w):
    return pltpu.bitcast(w, BF16)


def _combine(quad, spec):
    p, sign, q = spec
    if not sign:
        return quad(p)
    x, y = quad(p).astype(F32), quad(q).astype(F32)
    return x + y if sign > 0 else x - y


def _strassen(prod, emit, order):
    acc = {}
    for n, i in enumerate(order):
        m = prod(i)
        for q, terms in enumerate(_OUT):
            if i not in terms:
                continue
            if q not in acc:
                acc[q] = (terms[i], m)
            elif acc[q][0] == terms[i]:
                acc[q] = (terms[i], acc[q][1] + m)
            else:
                acc[q] = (1, acc[q][1] - m if terms[i] < 0 else m - acc[q][1])
            if all(t in order[:n + 1] for t in terms):
                emit(q, acc[q][1])


def _product(a, b, split, strip, order):
    if not split:
        return _dot(a.astype(BF16), b.astype(BF16))
    (m, k), n = a.shape, b.shape[1]
    mh, kh, nh = m // 2, k // (2 * LANE) * LANE, n // (2 * LANE) * LANE
    af, bf = a.astype(F32), b.astype(F32)

    def aq(q):
        return af[(q // 2) * mh:(q // 2 + 1) * mh, (q % 2) * kh:(q % 2 + 1) * kh]

    left = [_combine(aq, spec).astype(BF16) for spec in _LHS]
    quads = [[] for _ in range(4)]
    for c in range(0, nh, strip):
        def bq(q):
            return bf[(q // 2) * kh:(q // 2 + 1) * kh, (q % 2) * nh + c:(q % 2) * nh + c + strip]

        _strassen(lambda i: _dot(left[i], _combine(bq, _RHS[i]).astype(BF16)),
                  lambda q, v: quads[q].append(v), order)
    r = jnp.concatenate([jnp.concatenate(quads[0] + quads[1], axis=1),
                         jnp.concatenate(quads[2] + quads[3], axis=1)], axis=0)
    if 2 * kh < k:
        r = r + _dot(a[:, 2 * kh:].astype(BF16), b[2 * kh:, :2 * nh].astype(BF16))
    if 2 * nh < n:
        r = jnp.concatenate([r, _dot(a.astype(BF16), b[:, 2 * nh:].astype(BF16))], axis=1)
    return r


def _each(n, fn):
    def body(i, carry):
        fn(i)
        return carry

    lax.fori_loop(0, n, body, 0)


def _make_kernel(S, D, H, E, M, L, F):
    DM = (D // LANE) * LANE
    DR = D - DM
    DP = DM + LANE
    NT = DM // LANE
    NP = H // 2
    HG = H // 2
    PG = HG // 2
    R = M + L
    KT = H * R // LANE
    WB = NT * NP + NP // 2
    NB = S // LANE
    SB = LANE // L
    DH, FH, SH = D // 2, F // 2, S // 2
    SC = 2 * LANE
    NJ = SH // SC
    assert (D, H, E, M, R) == (448, 16, 2 * LANE, 8, 40) and S % (4 * SC) == 0 and F % (2 * LANE) == 0

    TILE = ((0, 1, 4), (2, 3, 5), (8, 9, 12), (10, 11, 13), (6, 7, 14))
    LAST = H - 1
    KPAIR = ((2, 0), (3, 1), (5, 4), (7, 6))
    KPOS = {g * HG + j: (g * PG + i, half)
            for g in range(2) for i, pr in enumerate(KPAIR) for half, j in enumerate(pr)}
    K_CHUNKS = ((2 * LANE, D - 2 * LANE), (0, 2 * LANE))

    def kernel(xt_hbm, mem0_hbm, wq_hbm, wk_hbm, wv_hbm, wo_hbm, w1_hbm, b1_hbm, w2_hbm, b2_hbm,
               out_hbm,
               raw, raw_k, wo_v, sw, sk, wu, wz, wt, wb, xt_v, xn, o_v, ht_v, hn_v,
               w1_v, w2_v, g_v, out_v, mem0_v, b1_v, b2_v, b2f_v,
               sems, sem_r, sem_o, sem_k):
        def heads(g):
            return pl.ds(pl.multiple_of(g * HG, HG), HG)

        def tokens(b):
            return pl.ds(b * LANE if isinstance(b, int) else pl.multiple_of(b * LANE, LANE), LANE)

        def cp_v(g):
            return pltpu.make_async_copy(wv_hbm.at[:, heads(g), :], raw.at[g], sem_r.at[g])

        def cp_q(g):
            return pltpu.make_async_copy(wq_hbm.at[:, heads(g), :], raw.at[2 + g], sem_r.at[2 + g])

        def cp_k(g, c):
            rows = pl.ds(*K_CHUNKS[c])
            return pltpu.make_async_copy(wk_hbm.at[rows, heads(g), :], raw_k.at[g, rows], sem_k.at[2 * g + c])

        def cp_o(p):
            return pltpu.make_async_copy(wo_hbm.at[pl.ds(2 * p, 2)], wo_v.at[pl.ds(2 * p, 2)], sem_o.at[p])

        def cp_x(b, sem):
            return pltpu.make_async_copy(xt_hbm.at[:, tokens(b)], xt_v.at[b], sem)

        def cp_w2(j, half):
            return pltpu.make_async_copy(w2_hbm.at[:, pl.ds(half * SH + j * SC, SC)],
                                         w2_v.at[j, :, pl.ds(half * SC, SC)], sems.at[4])

        def cp_out(q, j):
            rows = pl.ds((q // 2) * DH, DH)
            n0 = j * SC if isinstance(j, int) else pl.multiple_of(j * SC, SC)
            return pltpu.make_async_copy(out_v.at[j, rows, pl.ds((q % 2) * SC, SC)],
                                         out_hbm.at[rows, pl.ds((q % 2) * SH + n0, SC)], sems.at[2])

        def wait_filled(buf, sem):
            pltpu.make_async_copy(buf, buf, sem).wait()

        def start_values(g):
            cp_v(g).start()
            _each(PG, lambda pp: cp_o(g * PG + pp).start())

        def start_keys(g):
            cp_q(g).start()
            _each(len(K_CHUNKS), lambda i: [pl.when(i == c)(cp_k(g, c).start) for c in range(len(K_CHUNKS))])
            pl.when(g == 0)(cp_x(0, sems.at[3]).start)

        _each(2, start_values)
        _each(2, start_keys)
        small = [pltpu.make_async_copy(src, dst, sems.at[0])
                 for src, dst in ((mem0_hbm, mem0_v), (b1_hbm, b1_v), (b2_hbm, b2_v))]
        for cp in small:
            cp.start()
        _each(NB - 1, lambda i: cp_x(i + 1, sems.at[5]).start())
        cp_w1 = pltpu.make_async_copy(w1_hbm, w1_v, sems.at[1])
        cp_w1.start()
        for j in range(NJ):
            for half in range(2):
                cp_w2(j, half).start()

        low = lax.broadcasted_iota(jnp.int32, (1, LANE), 1) < DR
        halves = (_lo_f32, _hi_f32)
        o_v[0:LANE, :] = jnp.zeros((LANE, DP), F32)

        def relayout(src, dst, d0, nd):
            for d in range(d0, d0 + nd, DR):
                u = pltpu.bitcast(src[d:d + DR].reshape(DR * HG, E), U32)
                dst[0, d * PG:(d + DR) * PG, :] = u[:, :LANE]
                dst[1, d * PG:(d + DR) * PG, :] = u[:, LANE:]

        def pair(src, pp, d0, nd, step=1):
            idx = pl.ds(d0 * PG + pp, nd, stride=step * PG)
            return jnp.concatenate([src[0, idx, :], src[1, idx, :]], axis=1)

        def store_main(dst, g, j, d0, w):
            rows = pl.ds(d0 // 2, w.shape[0])
            for t in range(NT):
                dst[t * NP + g * PG + j // 2, rows, (j % 2) * LANE:(j % 2 + 1) * LANE] = w[:, t * LANE:(t + 1) * LANE]

        def store_rem(dst, g, i, d0, w):
            rows = pl.ds(d0 // 2, w.shape[0])
            dst[NT * NP + g * (PG // 2) + i // 2, rows, (i % 2) * LANE:(i % 2 + 1) * LANE] = w

        def fold_values(g):
            rem = {}
            for j in range(HG):
                pp, par = divmod(j, 2)
                p = g * PG + pp
                for i in {0: (0,), 2: (1,), 4: (2, 3)}.get(j, ()):
                    cp_o(g * PG + i).wait()
                if par == 0:
                    words = [pair(sw.at[g], pp, i, DH, 2) for i in range(2)]
                if j == HG - 1:
                    wait_filled(raw.at[g + 1], sem_r.at[g + 1])
                even, odd = map(halves[par], words)
                o = wo_v[2 * p + par]

                def edge():
                    rem[j] = _dot_nt(o[DM:], jnp.concatenate([even, odd, odd[:DR]], axis=0).astype(BF16))
                    for i, hs in enumerate(KPAIR):
                        if j == max(hs):
                            tile = jnp.concatenate([rem[h] for h in hs], axis=0).T
                            tile = _interleave(tile[:DH], tile[DH:D])
                            store_rem(wz, g, i, 0, tile[:DM // 2])
                            t0 = tile[DM // 2:]
                            t1 = pltpu.roll(t0, DR, 1)
                            for h, both in zip(hs, (jnp.where(low, t0, t1), jnp.where(low, t1, t0))):
                                wb[g * PG + h // 2, (h % 2) * (DR // 2):(h % 2 + 1) * (DR // 2), DM:] = both

                edge_last = j in (0, 2, 4)
                if not edge_last:
                    edge()
                r = _interleave(_dot_nt(even, o[:DM]), _dot_nt(odd, o[:DM]))
                if j == HG - 1:
                    relayout(raw.at[g + 1], sw.at[1 - g], 0, D)
                store_main(wz, g, j, 0, r[:DM // 2])
                wb[p, par * (DR // 2):(par + 1) * (DR // 2), :DM] = r[DM // 2:]
                if edge_last:
                    edge()

        def norm_input(b):
            xv = _layernorm_t(xt_v[b].astype(F32))
            xn[tokens(b), :] = jnp.concatenate([xv, xv[DM:]], axis=0).T

        def fold_keys(g):
            def fetch(c):
                cp_k(g, c).wait()
                relayout(raw_k.at[g], sk, *K_CHUNKS[c])

            query = {}
            for c, (d0, nd) in enumerate(K_CHUNKS):
                nm = min(nd, DM - d0)
                rem = {}
                for pp in range(PG):
                    if c == 0 and pp == 0:
                        fetch(0)
                    if c == 0 and pp == PG - 1:
                        fetch(1)
                    words = [pair(sk, pp, d0 + i, nm // 2, 2) for i in range(2)]
                    if c == 0:
                        wq = pair(sw.at[g], pp, 0, D)
                        for par, half in enumerate(halves):
                            q = half(wq)
                            query[2 * pp + par] = q[:DM].astype(BF16), q[DM:]
                    tail = []
                    if nm < nd:
                        wr = pair(sk, pp, DM, DR)
                        for par, half in enumerate(halves):
                            qm, qr = query[2 * pp + par]
                            rhs = jnp.concatenate([qm, jnp.concatenate([qr, qr], axis=0).astype(BF16)], axis=0)
                            tail.append(_dot_nt(half(wr), rhs))

                    def edge(par):
                        j = 2 * pp + par
                        k = jnp.concatenate([halves[par](w) for w in words], axis=0)
                        rem[j] = _dot_nt(query[j][1], k.astype(BF16))
                        for i, hs in enumerate(KPAIR):
                            if j == max(hs):
                                tile = jnp.concatenate([rem[h] for h in hs], axis=0).T
                                store_rem(wu, g, i, d0, _interleave(tile[:nm // 2], tile[nm // 2:]))

                    def body(par):
                        j = 2 * pp + par
                        store_main(wu, g, j, d0, _interleave(*(_dot_nt(halves[par](w), query[j][0]) for w in words)))

                    body(0)
                    edge(0)
                    edge(1)
                    body(1)
                    if tail:
                        wt[g * (PG // 2) + pp // 2, :, (pp % 2) * LANE:(pp % 2 + 1) * LANE] = _pack(
                            jnp.concatenate(tail, axis=0).T[:D])

            @pl.when(g == 0)
            def _():
                cp_q(1).wait()
                cp_x(0, sems.at[3]).wait()
                relayout(raw.at[3], sw.at[1], 0, D)
                norm_input(0)

        cp_v(0).wait()
        relayout(raw.at[0], sw.at[0], 0, D)
        _each(2, fold_values)
        _each(2, fold_keys)

        def project(ha, w_ref, t):
            base, n = (t * NP, NP) if t < NT else (NT * NP, NP // 2)
            out = []
            for p0 in range(0, n, 4):
                r = _dot(ha, _unpack(jnp.concatenate([w_ref[base + p0 + i] for i in range(4)], axis=1)))
                out += [r[:, i * LANE:(i + 1) * LANE] for i in range(8)]
            return out

        def main_blocks(ha, w_ref, t):
            hd = project(ha, w_ref, t)
            return [jnp.concatenate([hd[h] for h in TILE[k]] + [hd[LAST][k * M:(k + 1) * M]], axis=0)
                    for k in range(KT)]

        def rem_blocks(ha, w_ref, rr):
            rem = project(ha, w_ref, NT)
            blocks = []
            for k in range(KT):
                own = TILE[k][2] % 2
                mine = low if own == 0 else jnp.logical_not(low)

                def part(h):
                    i, half = KPOS[h]
                    v = rem[i][k * M:(k + 1) * M] if h == LAST else rem[i]
                    if half == own:
                        v = pltpu.roll(v, DR, 1)
                    return jnp.where(mine, rr if h == TILE[k][2] else 0.0, v)

                blocks.append(jnp.concatenate([part(h) for h in TILE[k] + (LAST,)], axis=0))
            return blocks

        scale = float(E) ** -0.5
        key = lax.broadcasted_iota(jnp.int32, (R, 3 * R), 0)
        col = lax.broadcasted_iota(jnp.int32, (R, 3 * R), 1)
        qry = col - jnp.where(col >= R, R, 0) - jnp.where(col >= 2 * R, R, 0)
        grp = lax.broadcasted_iota(jnp.int32, (M, 3 * R), 1)

        def softmax_keys(v):
            v = jnp.where((qry < M) | (qry >= key), v, MASKED / scale)
            e = jnp.exp2((v - jnp.max(v, axis=0, keepdims=True)) * (scale * LOG2E))
            return e * (1.0 / jnp.sum(e, axis=0, keepdims=True))

        def shift(v, n):
            if n == 0:
                return v
            v = jnp.concatenate([v, jnp.zeros((M, LANE - 3 * R), F32)], axis=1)
            return pltpu.roll(v, n % LANE, 1)[:, :3 * R]

        def step(s, mem, side):
            rows = pl.ds(pl.multiple_of(s * L, L), L)
            hh = jnp.concatenate([mem, xn[rows, :]], axis=0)
            ha, rr = hh[:, :DM], hh[:, DM:]
            own = jnp.concatenate([jnp.where(low, rr, 0.0), jnp.where(low, 0.0, rr),
                                   jnp.zeros((LANE - 2 * R, LANE), F32)], axis=0)
            own_t = own.T
            side()

            kb, tq = {}, {}
            for t in (0, NT, 1, 2):
                kb[t] = [b.T for b in (main_blocks(ha, wu, t) if t < NT else rem_blocks(ha, wu, rr))]
            for t in (1, 0):
                r = _dot(hh[:, :D], _unpack(jnp.concatenate([wt[2 * t], wt[2 * t + 1]], axis=1)))
                for i in range(4):
                    tq[4 * t + i] = r[:, i * LANE:(i + 1) * LANE]
            vrem = rem_blocks(ha, wz, rr)
            sc = [None] * (KT + 1)
            for k in (3, 4, KT, 0, 1, 2):
                if k == KT:
                    sc[k] = _dot(tq[LAST // 2], own_t.astype(BF16))
                    continue
                i, half = divmod(TILE[k][2], 2)
                third = jnp.where(low, tq[i], rr) if half == 0 else jnp.where(low, rr, tq[i])
                rhs = jnp.concatenate([jnp.concatenate([kb[t][k] for t in range(NT)], axis=0), kb[NT][k], own_t], axis=0)
                sc[k] = _dot(jnp.concatenate([ha, third, tq[TILE[k][0] // 2]], axis=1), rhs.astype(BF16))
            vb = [main_blocks(ha, wz, t) for t in range(NT)]

            sa = jnp.concatenate(sc[:3], axis=0).T
            sb = jnp.concatenate(sc[3:], axis=0).T
            g1, g3 = grp < R, grp >= 2 * R
            tail = [(sa if k < 3 else sb)[3 * R:] for k in range(KT)]
            home = sb[R:2 * R] + jnp.concatenate(
                [jnp.where(g3, shift(tail[k], (2 - k % 3) * R), 0.0) for k in range(KT)], axis=0)
            ps = [softmax_keys(v) for v in (sa[0:R], sa[R:2 * R], sa[2 * R:3 * R], sb[0:R], home, sb[2 * R:3 * R])]
            back = [shift(ps[4][k * M:(k + 1) * M], (k % 3 - 2) * R) for k in range(KT)]
            ta = jnp.where(g1, back[0], jnp.where(g3, back[2], back[1]))
            tb = jnp.where(g1, back[3], back[4])
            pa = jnp.concatenate(ps[:3] + [ta], axis=0).T
            pb = jnp.concatenate(ps[3:] + [tb], axis=0).T
            pm = [pa[i * R:(i + 1) * R] for i in range(3)] + [pb[i * R:(i + 1) * R] for i in range(2)]

            ra, rb = _dot(pa, own.astype(BF16)), _dot(pb, own.astype(BF16))
            xa = [ra[i * R:(i + 1) * R] for i in range(3)] + [rb[i * R:(i + 1) * R] for i in range(2)]
            xb = [_dot(pm[k], vrem[k].astype(BF16)) for k in range(KT)]
            rhs = jnp.concatenate([jnp.concatenate([vb[t][k] for t in range(NT)], axis=1) for k in range(KT)], axis=0)
            oa = _dot(jnp.concatenate(pm, axis=1), rhs.astype(BF16))
            single = {TILE[k][2]: xb[k] for k in range(KT)}
            single[LAST] = rb[2 * R:]
            both = {TILE[k][0] // 2: xa[k] for k in range(KT)}
            pr = [both[p] if p in both else jnp.where(low, single[2 * p], single[2 * p + 1]) for p in range(NP)]
            ob = _dot(jnp.concatenate(pr, axis=1), _unpack(jnp.concatenate([wb[p] for p in range(NP)], axis=0)))
            hi_sum, lo_sum = (functools.reduce(jnp.add, [xb[k] for k in range(KT) if TILE[k][2] % 2 == half])
                              for half in range(2))
            orem = jnp.where(low, lo_sum, hi_sum)
            o = ob + jnp.concatenate([oa, orem + pltpu.roll(orem, DR, 1)], axis=1)
            o_v[rows, :] = o[M:]
            return o[:M]

        def norm_output(b):
            ht = xt_v[b].astype(F32) + o_v[tokens(b), :].T[:D]
            ht_v[b] = ht
            hn_v[b] = _layernorm_t(_layernorm_t(ht), 0.5)

        def block(b, mem):
            def side():
                norm_output(jnp.maximum(b - 1, 0))
                norm_input(jnp.minimum(b + 1, NB - 1))

            for j in range(SB):
                mem = step(b * SB + j, mem, side if j == 1 else lambda: None)
            return mem

        for cp in small:
            cp.wait()
        wait_filled(xt_v.at[pl.ds(1, NB - 1)], sems.at[5])
        m0 = mem0_v[...].astype(F32)
        lax.fori_loop(0, NB, block, jnp.concatenate([m0, m0[:, DM:]], axis=1))
        cp_w1.wait()
        wait_filled(w2_v, sems.at[4])

        norm_output(NB - 1)
        b1f = 0.5 * b1_v[...].astype(F32).reshape(1, F)
        b2f = b2_v[...].astype(F32).reshape(1, S)
        for i in range(NB):
            b2f_v[i] = b2f[:, i * LANE:(i + 1) * LANE]

        def hq(q):
            return jnp.concatenate([hn_v[(q % 2) * (NB // 2) + i, (q // 2) * DH:(q // 2 + 1) * DH, :]
                                    for i in range(NB // 2)], axis=1)

        def w1q(q):
            return w1_v[(q // 2) * SH:(q // 2 + 1) * SH, (q % 2) * FH:(q % 2 + 1) * FH]

        gq = {}

        def activate(q, v):
            gq[q] = _gelu_of_half(v + b1f[:, (q % 2) * FH:(q % 2 + 1) * FH])
            for i, (qa, sign, qb) in enumerate(_LHS):
                need = (qa, qb) if sign else (qa,)
                if q in need and all(n in gq for n in need):
                    g_v[i] = _combine(gq.get, _LHS[i])

        _strassen(lambda i: _product(_combine(hq, _LHS[i]), _combine(w1q, _RHS[i]), i in (1, 3, 4),
                                     LANE, (1, 3, 4, 2, 0, 5, 6)),
                  activate, (2, 5, 4, 1, 3, 0, 6))

        def mlp2(j):
            def w2q(q):
                return w2_v[j, (q // 2) * FH:(q // 2 + 1) * FH, (q % 2) * SC:(q % 2 + 1) * SC]

            def finish(q, v):
                rows = slice((q // 2) * DH, (q // 2 + 1) * DH)
                first = (q % 2) * (NB // 2) + j * (SC // LANE)
                ht = jnp.concatenate([ht_v[first + i, rows, :] + b2f_v[first + i] for i in range(SC // LANE)], axis=1)
                out_v[j, rows, (q % 2) * SC:(q % 2 + 1) * SC] = (ht + v).astype(BF16)
                cp_out(q, j).start()

            _strassen(lambda i: _product(g_v[i], _combine(w2q, _RHS[i]), i != 0, LANE, (1, 3, 2, 4, 0, 6, 5)),
                      finish, (1, 3, 4, 2, 0, 5, 6))

        _each(NJ // 2, lambda t: [mlp2(2 * t + n) for n in range(2)])
        for j in range(NJ):
            for q in range(4):
                cp_out(q, j).wait()

    words = D * PG + 32
    scratch = [
        pltpu.VMEM((4, D, HG, E), BF16), pltpu.VMEM((2, D, HG, E), BF16), pltpu.VMEM((H, D, E), BF16),
        pltpu.VMEM((2, 2, words, LANE), U32), pltpu.VMEM((2, words, LANE), U32),
        pltpu.VMEM((WB, DM // 2, 2 * LANE), U32), pltpu.VMEM((WB, DM // 2, 2 * LANE), U32),
        pltpu.VMEM((NP // 2, DH, 2 * LANE), U32), pltpu.VMEM((NP, LANE // 2, DP), U32),
        pltpu.VMEM((NB, D, LANE), BF16), pltpu.VMEM((S, DP), F32), pltpu.VMEM((S, DP), F32),
        pltpu.VMEM((NB, D, LANE), F32), pltpu.VMEM((NB, D, LANE), F32),
        pltpu.VMEM((S, F), BF16), pltpu.VMEM((NJ, F, 2 * SC), BF16),
        pltpu.VMEM((7, DH, FH), F32), pltpu.VMEM((NJ, D, 2 * SC), BF16),
        pltpu.VMEM((M, D), BF16), pltpu.VMEM((F,), BF16), pltpu.VMEM((S,), BF16), pltpu.VMEM((NB, 1, LANE), F32),
        pltpu.SemaphoreType.DMA((6,)), pltpu.SemaphoreType.DMA((4,)), pltpu.SemaphoreType.DMA((NP,)),
        pltpu.SemaphoreType.DMA((4,)),
    ]
    return kernel, scratch


@functools.partial(jax.jit, static_argnames=("A_seg_len",))
def pallas_sequential_preLN__memory_aug_recurrent_mem_tr__mixer_token_mlp__prompt_kernel(
        A_x, A_mem0, A_Wq, A_Wk, A_Wv, A_Wo, A_seg_len, B_x, B_w1, B_b1, B_w2, B_b2):
    del B_x
    _, S, D = A_x.shape
    _, H, E = A_Wq.shape
    M = A_mem0.shape[1]
    F = B_w1.shape[1]
    kernel, scratch = _make_kernel(S, D, H, E, M, A_seg_len, F)
    hbm = pl.BlockSpec(memory_space=pltpu.HBM)
    out = pl.pallas_call(
        kernel,
        out_shape=pltpu.HBM((D, S), A_x.dtype),
        in_specs=[hbm] * 10,
        out_specs=hbm,
        scratch_shapes=scratch,
        compiler_params=pltpu.CompilerParams(vmem_limit_bytes=110 * 1024 * 1024),
    )(A_x.reshape(S, D).T, A_mem0.reshape(M, D), A_Wq, A_Wk, A_Wv, A_Wo.transpose(0, 2, 1),
      B_w1, B_b1, B_w2, B_b2)
    return out.T.reshape(A_x.shape)
```
